```python
import jax
import jax.numpy as jnp

def _softmax(x, axis=-1):
    return jax.nn.softmax(x, axis=axis)
def _gelu(x):
    return jax.nn.gelu(x, approximate=True)
def _silu(x):
    return jax.nn.silu(x)
def _sigmoid(x):
    return jax.nn.sigmoid(x)
def _layernorm(x, axis=-1, eps=1e-5):
    m = jnp.mean(x, axis=axis, keepdims=True)
    v = jnp.var(x, axis=axis, keepdims=True)
    return (x - m) / jnp.sqrt(v + eps)
def _scatter_add(tgt, idx, src, axis=0):
    return tgt.at[idx].add(src)
def _segment_sum(src, seg, n):
    return jax.ops.segment_sum(src, seg, n)
class _Rng:
    def __init__(self, key):
        self._k = key
    def _next(self):
        self._k, sub = jax.random.split(self._k)
        return sub
    def normal(self, shape):
        return jax.random.normal(self._next(), shape, dtype=jnp.bfloat16)
    def randint(self, lo, hi, shape):
        return jax.random.randint(self._next(), shape, lo, hi, dtype=jnp.int32)
    def uniform(self, shape, lo=0.0, hi=1.0):
        return jax.random.uniform(self._next(), shape, jnp.bfloat16, lo, hi)
    def permutation(self, n):
        return jax.random.permutation(self._next(), n)


kernel_name = 'sequential_preLN__mha_block_cached__moe_arch_mod__decode'

def setup_inputs():
    _rng = _Rng(jax.random.key(int.from_bytes(__import__("os").urandom(4), "little")))
    _w = (lambda a: (lambda t: t.astype(jnp.bfloat16) if jnp.issubdtype(t.dtype, jnp.floating) else t)(jnp.asarray(a)))
    def _A_setup():
        B, Sq, D = 4, 1, 640
        H, Sk, Dh = 32, 8192, 192
        return {
            "x": _w((lambda *s: _rng.normal(s) * 0.05)(B, Sq, D)),
            "k_cache": _w((lambda *s: _rng.normal(s) * 0.05)(B, H, Sk, Dh)),
            "v_cache": _w((lambda *s: _rng.normal(s) * 0.05)(B, H, Sk, Dh)),
            "wq": _w((lambda *s: _rng.normal(s) * 0.05)(D, H * Dh) * (D ** -0.5)),
            "wo": _w((lambda *s: _rng.normal(s) * 0.05)(H * Dh, D) * ((H * Dh) ** -0.5)),
        }
    _A_in = _A_setup()

    def _B_setup():
        B, S, D, F, C = 4, 1, 640, 1536, 1
        return {
            "x": _w((lambda *s: _rng.normal(s) * 0.05)(B, S, D)),
            "w_r": _w((lambda *s: _rng.normal(s) * 0.05)(D)),
            "w_gate": _w((lambda *s: _rng.normal(s) * 0.05)(D, F)),
            "w_up": _w((lambda *s: _rng.normal(s) * 0.05)(D, F)),
            "w_down": _w((lambda *s: _rng.normal(s) * 0.05)(F, D)),
        }
    _B_in = _B_setup()

    return {
        "A_x": _A_in["x"],
        "A_k_cache": _A_in["k_cache"],
        "A_v_cache": _A_in["v_cache"],
        "A_wq": _A_in["wq"],
        "A_wo": _A_in["wo"],
        "B_x": _B_in["x"],
        "B_w_r": _B_in["w_r"],
        "B_w_gate": _B_in["w_gate"],
        "B_w_up": _B_in["w_up"],
        "B_w_down": _B_in["w_down"],
    }

def reference(A_x, A_k_cache, A_v_cache, A_wq, A_wo, B_x, B_w_r, B_w_gate, B_w_up, B_w_down):
    def _A_ref(x, k_cache, v_cache, wq, wo):
        B, Sq, D = x.shape
        H, Dh = 32, 192
        q = (lambda x, *d: x.transpose(*d))((x @ wq).reshape(B, Sq, H, Dh), 0, 2, 1, 3)
        scores = jnp.einsum("bhqd,bhkd->bhqk", q, k_cache) * (Dh ** -0.5)
        p = _softmax(scores, axis=-1)
        o = jnp.einsum("bhqk,bhkd->bhqd", p, v_cache)
        return (lambda x, *d: x.transpose(*d))(o, 0, 2, 1, 3).reshape(B, Sq, H * Dh) @ wo

    def _B_ref(x, w_r, w_gate, w_up, w_down):
        B, S, D = x.shape
        C = 1
        r = x @ w_r
        idx = jnp.argsort(-r, axis=-1)[:, :C]
        idx_e = jnp.repeat(idx.reshape(B, C, 1), D, axis=2)
        x_sel = jnp.take_along_axis(x, idx_e, axis=1)
        g = _silu(x_sel @ w_gate)
        u = x_sel @ w_up
        y = (g * u) @ w_down
        r_sel = _sigmoid(jnp.take_along_axis(r, idx, axis=1))
        y = y * r_sel.reshape(B, C, 1)
        b_off = (jnp.arange(B) * S).reshape(B, 1)
        flat_idx = (idx + b_off).reshape(B * C)
        zero = (x * 0.0).reshape(B * S, D)
        upd = _scatter_add(zero, flat_idx, y.reshape(B * C, D), axis=0)
        return x + upd.reshape(B, S, D)

    x = A_x
    h = x + _A_ref(_layernorm(x, axis=-1), A_k_cache, A_v_cache, A_wq, A_wo)
    h2 = h + _B_ref(_layernorm(h, axis=-1), B_w_r, B_w_gate, B_w_up, B_w_down)
    return h2
```

```python
import functools

import jax
import jax.numpy as jnp
import jax.experimental.pallas as pl
import jax.experimental.pallas.tpu as pltpu

_EPS = 1e-5
_HG = 8
_RB = 64
_NR = 8
_CW = 256
CFG = dict(compute=True, wq=(4, 512), wo=(4, 640), gu=(8, 256), wd=(4, 640), fw=256)


def _layernorm(x):
    m = jnp.mean(x, axis=-1, keepdims=True)
    d = x - m
    v = jnp.mean(d * d, axis=-1, keepdims=True)
    return d / jnp.sqrt(v + _EPS)


def _dot(a, b):
    return jnp.dot(a, b, preferred_element_type=jnp.float32)


def _dot_nt(a, b):
    return jax.lax.dot_general(
        a, b, (((1,), (1,)), ((), ())), preferred_element_type=jnp.float32
    )


def _wait_all(buf, sem):
    pltpu.make_async_copy(buf, buf, sem).wait()


def _loop(lo, hi, fn):
    jax.lax.fori_loop(lo, hi, lambda i, c: fn(i), None)


def _body(
    x_hbm, kt_hbm, vt_hbm, wq_hbm, wo_hbm, wr_hbm, wg_hbm, wu_hbm, wd_hbm,
    out_ref,
    cbuf, wqbuf, wobuf, wgbuf, wubuf, wdbuf, xbuf, wrbuf,
    q_scr, qd_scr, s_scr, p_scr, l_scr, acc_scr, o_scr, h_scr,
    csem, wsem, dsem,
    *, B, H, Dh, Sk, D, F, cfg,
):
    P = _HG * Dh
    BR = _NR * _RB
    n_hg = H // _HG
    n_groups = B * n_hg
    NS = _RB // 8
    scale = Dh ** -0.5
    bf16 = jnp.bfloat16
    FW = cfg["fw"]

    def issue_cache(g, blocks, i):
        rows = pl.ds(pl.multiple_of(i * 8, 8), 8)
        for c in range(0, Sk, _CW):
            for queue, blk in enumerate(blocks):
                src = kt_hbm if blk < 3 else vt_hbm
                pltpu.make_async_copy(
                    src.at[g * 3 + blk % 3, :, rows, pl.ds(c, _CW)],
                    cbuf.at[blk, :, rows, pl.ds(c, _CW)],
                    csem.at[blk],
                ).start(priority=queue)

    def issue_halves(src, dst, sem, cw, i):
        rows = pl.ds(pl.multiple_of(i * 8, 8), 8)
        n = src.shape[0] // 2
        for c in range(0, src.shape[2], cw):
            w = min(cw, src.shape[2] - c)
            for queue in range(2):
                idx = (pl.ds(queue * n, n), rows, pl.ds(c, w))
                pltpu.make_async_copy(src.at[idx], dst.at[idx], sem).start(priority=queue)

    def issue_gate_up(i):
        rows = pl.ds(pl.multiple_of(i * 8, 8), 8)
        cw = cfg["gu"][1]
        for c in range(0, F, cw):
            idx = (slice(None), rows, pl.ds(c, cw))
            pltpu.make_async_copy(wg_hbm.at[idx], wgbuf.at[idx], wsem.at[2]).start(priority=0)
            pltpu.make_async_copy(wu_hbm.at[idx], wubuf.at[idx], wsem.at[3]).start(priority=1)

    def issue_down(f):
        n = FW // 32
        for i in range(n):
            r = (i % 2) * (FW // 2) + (i // 2) * 32
            pltpu.make_async_copy(
                wd_hbm.at[f, pl.ds(r, 32), :], wdbuf.at[f, pl.ds(r, 32), :], dsem.at[f]
            ).start(priority=i % 2)

    x_cp = pltpu.make_async_copy(x_hbm, xbuf, wsem.at[4])
    wr_cp = pltpu.make_async_copy(wr_hbm, wrbuf, wsem.at[5])
    _loop(0, 1, lambda i: issue_halves(wq_hbm, wqbuf, wsem.at[0], cfg["wq"][1], i))
    x_cp.start()
    wr_cp.start(priority=1)
    _loop(1, wq_hbm.shape[1] // 8, lambda i: issue_halves(wq_hbm, wqbuf, wsem.at[0], cfg["wq"][1], i))

    x_cp.wait()
    x4 = xbuf[...].astype(jnp.float32)
    x = jnp.concatenate([x4, x4], axis=0)
    xn = _layernorm(x).astype(bf16)
    row = jax.lax.broadcasted_iota(jnp.int32, (_HG, P), 0)
    col = jax.lax.broadcasted_iota(jnp.int32, (_HG, P), 1)
    diag = (col >= row * Dh) & (col < row * Dh + Dh)
    o_scr[...] = jnp.zeros_like(o_scr)

    def block(blk, cols):
        return cbuf[blk, :, :, cols].reshape(BR, cols.size)

    def chunk(i, n):
        w = Sk // n
        return pl.ds(pl.multiple_of(i * w, w), w)

    n_wo = wo_hbm.shape[1] // 8 // (2 * NS)

    def issue(g, blocks, i, tail):
        @pl.when(g < n_groups)
        def _():
            issue_cache(g, blocks, i)

        if tail is not None:
            @pl.when(g == n_groups)
            def _():
                _loop(0, n_wo, lambda j: issue_halves(wo_hbm, wobuf, wsem.at[1], cfg["wo"][1], (tail * NS + i) * n_wo + j))

    def group(g):
        @pl.when(g > 0)
        def _():
            _wait_all(cbuf.at[2], csem.at[2])
            _wait_all(cbuf.at[3], csem.at[3])

        def scores_end(i):
            issue(g, (0, 1), i, 0)

            @pl.when((g > 0) & cfg["compute"])
            def _():
                cols = chunk(i, NS // 2)
                s = s_scr[:, cols] + _dot(qd_scr[:, 2 * BR:].astype(bf16), block(2, cols))
                s_scr[:, cols] = s * scale

        _loop(0, NS // 2, scores_end)

        @pl.when(g > 0)
        def _():
            s = s_scr[...]
            e = jnp.exp(s - jnp.max(s, axis=-1, keepdims=True))
            p_scr[...] = e
            l_scr[...] = jnp.sum(e, axis=-1, keepdims=True)
            acc_scr[...] = jnp.zeros_like(acc_scr)

        def values_start(i):
            issue(g, (0, 1), NS // 2 + i, 0)

            @pl.when((g > 0) & cfg["compute"])
            def _():
                cols = chunk(i, NS // 2)
                acc_scr[:, :BR] += _dot_nt(p_scr[:, cols].astype(bf16), block(3, cols))

        _loop(0, NS // 2, values_start)

        @pl.when(g > 0)
        def _():
            _wait_all(cbuf.at[4], csem.at[4])
            _wait_all(cbuf.at[5], csem.at[5])

        @pl.when(g == 0)
        def _():
            _wait_all(wqbuf, wsem.at[0])

        def values_end(i):
            issue(g, (2, 3), i, 1)

            @pl.when((g > 0) & cfg["compute"])
            def _():
                cols = chunk(i, NS)
                p = p_scr[:, cols].astype(bf16)
                acc_scr[:, BR:2 * BR] += _dot_nt(p, block(4, cols))
                acc_scr[:, 2 * BR:] += _dot_nt(p, block(5, cols))

            @pl.when((g == 0) & (i < n_hg))
            def _():
                cols = pl.ds(pl.multiple_of(i * P, P), P)
                q_scr[i] = _dot(xn, wqbuf[:, :, cols].reshape(D, P))

        _loop(0, NS, values_end)

        @pl.when(g > 0)
        def _():
            o = jnp.where(diag, acc_scr[...] / l_scr[...], 0.0)
            o_scr[(g - 1) % n_hg, pl.ds((g - 1) // n_hg, 1), :] = jnp.sum(o, axis=0, keepdims=True)

        @pl.when(g < n_groups)
        def _():
            _wait_all(cbuf.at[0], csem.at[0])
            _wait_all(cbuf.at[1], csem.at[1])
            qd_scr[...] = jnp.where(diag, q_scr[g % n_hg, pl.ds(g // n_hg, 1), :], 0.0)

            def scores_start(i):
                issue_cache(g, (4, 5), i)
                if cfg["compute"]:
                    cols = chunk(i, NS)
                    qd = qd_scr[:, :2 * BR].astype(bf16)
                    s_scr[:, cols] = _dot(qd[:, :BR], block(0, cols)) + _dot(qd[:, BR:], block(1, cols))

            _loop(0, NS, scores_start)

    _loop(0, n_groups + 1, group)

    n_gu = wg_hbm.shape[1] // 8
    _loop(0, n_gu // 2, issue_gate_up)
    _wait_all(wobuf, wsem.at[1])
    h_scr[...] = x
    nb = wobuf.shape[0] // n_hg
    rest = n_gu - n_gu // 2
    for i in range(n_hg):
        h_scr[...] += _dot(o_scr[i].astype(bf16), wobuf[i * nb:(i + 1) * nb].reshape(P, D))
        _loop(n_gu // 2 + rest * i // n_hg, n_gu // 2 + rest * (i + 1) // n_hg, issue_gate_up)
    _loop(0, F // FW, issue_down)

    h = h_scr[...]
    hn = _layernorm(h)
    hb = hn.astype(bf16)
    wr_cp.wait()
    r = jnp.sum(hn * wrbuf[...].astype(jnp.float32).reshape(1, D), axis=-1, keepdims=True)
    route = jax.nn.sigmoid(r)
    base = hn * 0.0
    _wait_all(wgbuf, wsem.at[2])
    _wait_all(wubuf, wsem.at[3])
    gate = _dot(hb, wgbuf[...].reshape(D, F))
    up = _dot(hb, wubuf[...].reshape(D, F))
    act = (gate * jax.nn.sigmoid(gate) * up).astype(bf16)
    y = jnp.zeros((2 * B, D), jnp.float32)
    for f in range(F // FW):
        _wait_all(wdbuf.at[f], dsem.at[f])
        y = y + _dot(act[:, f * FW:(f + 1) * FW], wdbuf[f])
    out = h + (hn + (base + y * route))
    out_ref[...] = out[:B].astype(out_ref.dtype)


def build(**kw):
    cfg = dict(CFG, **kw)

    def kernel(A_x, A_k_cache, A_v_cache, A_wq, A_wo, B_x, B_w_r, B_w_gate, B_w_up, B_w_down):
        del B_x
        B, Sq, D = A_x.shape
        _, H, Sk, Dh = A_k_cache.shape
        F = B_w_gate.shape[1]
        P = _HG * Dh
        assert Sq == 1 and B == 4 and H % _HG == 0 and P == 3 * _NR * _RB
        dt = A_k_cache.dtype
        f32 = jnp.float32
        kt = jnp.swapaxes(A_k_cache, 2, 3).reshape(-1, _NR, _RB, Sk)
        vt = jnp.swapaxes(A_v_cache, 2, 3).reshape(-1, _NR, _RB, Sk)
        wq = A_wq.reshape(2 * cfg["wq"][0], -1, H * Dh)
        wo = A_wo.reshape(2 * cfg["wo"][0], -1, D)
        wg = B_w_gate.reshape(cfg["gu"][0], -1, F)
        wu = B_w_up.reshape(cfg["gu"][0], -1, F)
        wd = B_w_down.reshape(-1, cfg["fw"], D)
        out = pl.pallas_call(
            functools.partial(_body, B=B, H=H, Dh=Dh, Sk=Sk, D=D, F=F, cfg=cfg),
            in_specs=[pl.BlockSpec(memory_space=pl.ANY)] * 9,
            out_specs=pl.BlockSpec(memory_space=pltpu.VMEM),
            out_shape=jax.ShapeDtypeStruct((B, D), A_x.dtype),
            scratch_shapes=[
                pltpu.VMEM((6, _NR, _RB, Sk), dt),
                pltpu.VMEM(wq.shape, dt),
                pltpu.VMEM(wo.shape, dt),
                pltpu.VMEM(wg.shape, dt),
                pltpu.VMEM(wu.shape, dt),
                pltpu.VMEM(wd.shape, dt),
                pltpu.VMEM((B, D), dt),
                pltpu.VMEM((D,), dt),
                pltpu.VMEM((H // _HG, 2 * B, P), f32),
                pltpu.VMEM((_HG, P), f32),
                pltpu.VMEM((_HG, Sk), f32),
                pltpu.VMEM((_HG, Sk), f32),
                pltpu.VMEM((_HG, 1), f32),
                pltpu.VMEM((_HG, P), f32),
                pltpu.VMEM((H // _HG, 2 * B, P), f32),
                pltpu.VMEM((2 * B, D), f32),
                pltpu.SemaphoreType.DMA((6,)),
                pltpu.SemaphoreType.DMA((6,)),
                pltpu.SemaphoreType.DMA((wd.shape[0],)),
            ],
            compiler_params=pltpu.CompilerParams(vmem_limit_bytes=100 * 1024 * 1024),
        )(A_x.reshape(B, D), kt, vt, wq, wo, B_w_r, wg, wu, wd)
        return out.reshape(B, Sq, D)

    return jax.jit(kernel)


pallas_sequential_preLN__mha_block_cached__moe_arch_mod__decode_kernel = build()
```

```python
import functools

import jax
import jax.numpy as jnp
import jax.experimental.pallas as pl
import jax.experimental.pallas.tpu as pltpu

_EPS = 1e-5
_HG = 8
_RB = 64
_NB = 8
_CW = 256
CFG = dict(compute=True, wq=(5, 384), wo=(4, 640), gu=(5, 512), wd=(768, 512, 256), dr=32, nb=True, ks=176, vs=40, ox=1, pw=1024)


def _layernorm(x):
    m = jnp.mean(x, axis=-1, keepdims=True)
    d = x - m
    v = jnp.mean(d * d, axis=-1, keepdims=True)
    return d / jnp.sqrt(v + _EPS)


def _dot(a, b):
    return jnp.dot(a, b, preferred_element_type=jnp.float32)


def _dot_nt(a, b):
    return jax.lax.dot_general(
        a, b, (((1,), (1,)), ((), ())), preferred_element_type=jnp.float32
    )


def _wait_all(buf, sem):
    pltpu.make_async_copy(buf, buf, sem).wait()


def _loop(lo, hi, fn):
    jax.lax.fori_loop(lo, hi, lambda i, carry: fn(i), None)


def _tile(i, n):
    return pl.ds(i * n if isinstance(i, int) else pl.multiple_of(i * n, n), n)


def _body(
    x_hbm, kt_hbm, vt_hbm, wq_hbm, wo_hbm, wr_hbm, wg_hbm, wu_hbm, wd_hbm,
    out_ref,
    cbuf, kfirst, vlast, wqbuf, wobuf, wgbuf, wubuf, wdbuf, xbuf, wrbuf,
    q_scr, qd_scr, s_scr, carry_scr, p_scr, l_scr, acc_scr, o_scr, h_scr,
    csem, wsem, dsem,
    *, B, H, Dh, Sk, D, F, cfg,
):
    P = _HG * Dh
    BR = _NB * _RB
    NS = _RB // 8
    n_hg = H // _HG
    n_groups = B * n_hg
    n_bands = kt_hbm.shape[0]
    scale = Dh ** -0.5
    bf16 = jnp.bfloat16
    KS, VS = cfg["ks"], cfg["vs"]

    def cache_copy(g, blk, i, cols, lo=0, hi=_NB):
        src, r = (kt_hbm, 8 * i + KS) if blk < 3 else (vt_hbm, 8 * i + _RB * _NB - VS)
        band = (g * 3 + blk % 3) * _NB + r // _RB - (0 if blk < 3 else _NB)
        return pltpu.make_async_copy(
            src.at[pl.ds(band + lo, hi - lo), _tile(r % _RB // 8, 8), cols],
            cbuf.at[blk, pl.ds(lo, hi - lo), _tile(i, 8), cols],
            csem.at[blk],
        )

    def issue_cache(g, blocks, i):
        for c in range(Sk // _CW):
            cols = _tile(c ^ ((c >> 2) & cfg["ox"]), _CW)
            for queue, blk in enumerate(blocks):
                cache_copy(g, blk, i, cols).start(priority=queue)

    def issue_edge(g, i):
        for j in range(NS):
            hi = _NB - (8 * j + KS) // _RB if g == n_groups - 1 else _NB
            lo = -((8 * j - VS) // _RB) if g == 0 else 0

            @pl.when(i == j)
            def _(j=j, lo=lo, hi=hi):
                def piece(c):
                    cache_copy(g, 2, j, _tile(c, _CW), 0, hi).start(priority=0)
                    cache_copy(g, 3, j, _tile(c, _CW), lo, _NB).start(priority=1)

                _loop(0, Sk // _CW, piece)

    def wait_rows(blk, n):
        _wait_all(cbuf.at[blk, pl.ds(0, n // _RB)], csem.at[blk])
        if n % _RB:
            _wait_all(cbuf.at[blk, 0, pl.ds(0, n % _RB)], csem.at[blk])

    def issue_k_first():
        for r in range(0, _RB, 8):
            n = -((r - KS) // _RB)

            def piece(c, r=r, n=n):
                for queue in range(2):
                    idx = (pl.ds(0, n), pl.ds(r, 8), _tile(c + queue * (Sk // cfg["pw"] // 2), cfg["pw"]))
                    pltpu.make_async_copy(kt_hbm.at[idx], kfirst.at[idx], wsem.at[6]).start(priority=queue)

            if n > 0:
                _loop(0, Sk // cfg["pw"] // 2, piece)

    def issue_v_last():
        def piece(c):
            for queue in range(2):
                rows, cols = pl.ds(_RB - VS, VS), _tile(c + queue * (Sk // 1024), 512)
                pltpu.make_async_copy(
                    vt_hbm.at[n_bands - 1, rows, cols], vlast.at[rows, cols], wsem.at[7]
                ).start(priority=queue)

        _loop(0, Sk // 1024, piece)

    def issue_halves(src, dst, sem, cw, i):
        n = src.shape[0] // 2
        for c in range(0, src.shape[2], cw):
            for queue in range(2):
                idx = (pl.ds(queue * n, n), _tile(i, 8), pl.ds(c, min(cw, src.shape[2] - c)))
                pltpu.make_async_copy(src.at[idx], dst.at[idx], sem).start(priority=queue)

    def issue_gate_up(i):
        cw = cfg["gu"][1]
        for c in range(0, F, cw):
            idx = (slice(None), _tile(i, 8), pl.ds(c, cw))
            pltpu.make_async_copy(wg_hbm.at[idx], wgbuf.at[idx], wsem.at[2]).start(priority=0)
            pltpu.make_async_copy(wu_hbm.at[idx], wubuf.at[idx], wsem.at[3]).start(priority=1)

    def down_copies():
        lo = 0
        for f, n in enumerate(cfg["wd"]):
            dr = cfg["dr"]
            for i in range(n // dr):
                rows = pl.ds(lo + (i % 2) * (n // 2) + (i // 2) * dr, dr)
                yield pltpu.make_async_copy(wd_hbm.at[rows, :], wdbuf.at[rows, :], dsem.at[f]), i % 2
            lo += n

    x_cp = pltpu.make_async_copy(x_hbm, xbuf, wsem.at[4])
    wr_cp = pltpu.make_async_copy(wr_hbm, wrbuf, wsem.at[5])
    issue_wq = functools.partial(issue_halves, wq_hbm, wqbuf, wsem.at[0], cfg["wq"][1])
    _loop(0, 2, issue_wq)
    x_cp.start()
    wr_cp.start(priority=1)
    kfirst[...] = jnp.zeros_like(kfirst)
    vlast[...] = jnp.zeros_like(vlast)
    cbuf[3, 0] = jnp.zeros((_RB, Sk), cbuf.dtype)
    _loop(2, wq_hbm.shape[1] // 8, issue_wq)
    issue_k_first()

    x_cp.wait()
    x4 = xbuf[...].astype(jnp.float32)
    x = jnp.concatenate([x4, x4], axis=0)
    xn = _layernorm(x).astype(bf16)
    row = jax.lax.broadcasted_iota(jnp.int32, (2 * _HG, P), 0)
    col = jax.lax.broadcasted_iota(jnp.int32, (2 * _HG, P), 1)
    k_diag = (col + KS >= row * Dh) & (col + KS < row * Dh + Dh)
    v_row = jnp.where(row < _HG, row, row - 2 * _HG)
    v_diag = (col - VS >= v_row * Dh) & (col - VS < v_row * Dh + Dh)
    p_scr[...] = jnp.zeros_like(p_scr)
    l_scr[...] = jnp.ones_like(l_scr)

    def block(blk, cols):
        return cbuf[blk, :, :, cols].reshape(BR, cols.size)

    n_wo = wo_hbm.shape[1] // 8
    n_gu = wg_hbm.shape[1] // 8
    T_WO = 11

    def issue_tail(t):
        u = jnp.maximum(t - T_WO, 0)
        v = jnp.maximum(t + 1 - T_WO, 0)
        _loop(
            jnp.minimum(t, T_WO) * n_wo // T_WO,
            jnp.minimum(t + 1, T_WO) * n_wo // T_WO,
            functools.partial(issue_halves, wo_hbm, wobuf, wsem.at[1], cfg["wo"][1]),
        )
        _loop(u * n_gu // (2 * NS - T_WO), v * n_gu // (2 * NS - T_WO), issue_gate_up)

    def group(g):
        started = (g > 0) & cfg["compute"]

        @pl.when((g > 0) & (g < n_groups))
        def _():
            wait_rows(2, BR)

        @pl.when(g == n_groups)
        def _():
            issue_v_last()
            wait_rows(2, BR - KS)

        pl.when(g > 1)(lambda: wait_rows(3, BR))
        pl.when(g == 1)(lambda: wait_rows(3, BR - VS))

        def issue_first(i):
            pl.when(g < n_groups)(lambda: issue_cache(g, (0, 1), i))
            pl.when(g == n_groups)(lambda: issue_tail(i))

        def scores_end(i):
            issue_first(i)

            @pl.when(started)
            def _():
                cols = _tile(i, 2 * Sk // NS)
                s_scr[:, cols] += _dot(qd_scr[:, 2 * BR:], block(2, cols))

        _loop(0, NS // 2, scores_end)

        @pl.when(started)
        def _():
            s = (s_scr[:_HG] + carry_scr[...]) * scale
            carry_scr[...] = s_scr[_HG:]
            e = jnp.exp(s - jnp.max(s, axis=-1, keepdims=True))
            e_prev = p_scr[...].astype(jnp.float32)[:_HG]
            p_scr[...] = jnp.concatenate([e, e_prev], axis=0).astype(bf16)
            l_scr[_HG:] = l_scr[:_HG]
            l_scr[:_HG] = jnp.sum(e, axis=-1, keepdims=True)
            acc_scr[...] = jnp.zeros_like(acc_scr)

        def values_start(i):
            issue_first(NS // 2 + i)

            @pl.when(started)
            def _():
                cols = _tile(i, 2 * Sk // NS)
                acc_scr[:, :BR] += _dot_nt(p_scr[:, cols], block(3, cols))

        _loop(0, NS // 2, values_start)

        @pl.when(g > 0)
        def _():
            wait_rows(4, BR)
            wait_rows(5, BR)

        @pl.when(g == 0)
        def _():
            _wait_all(wqbuf, wsem.at[0])

        @pl.when(g == n_groups - 1)
        def _():
            n = -(-KS // _RB)
            cbuf[2, _NB - n:] = jnp.zeros((n, _RB, Sk), cbuf.dtype)

        def values_end(i):
            pl.when((g > 0) & (g < n_groups - 1))(lambda: issue_cache(g, (2, 3), i))
            pl.when(g == 0)(lambda: issue_edge(0, i))
            pl.when(g == n_groups - 1)(lambda: issue_edge(n_groups - 1, i))
            pl.when(g == n_groups)(lambda: issue_tail(NS + i))

            @pl.when(started)
            def _():
                cols = _tile(i, Sk // NS)
                p = p_scr[:, cols]
                acc_scr[:, BR:2 * BR] += _dot_nt(p, block(4, cols))
                acc_scr[:, 2 * BR:] += _dot_nt(p, block(5, cols))

            @pl.when((g == 0) & (i < n_hg))
            def _():
                q = _dot(xn, wqbuf[:, :, _tile(i, P)].reshape(D, P))
                for b in range(B):
                    q_scr[pl.ds(b * n_hg + i, 1), :] = q[b:b + 1]

        _loop(0, NS, values_end)

        @pl.when(started)
        def _():
            o = jnp.where(v_diag, acc_scr[...] / l_scr[...], 0.0)
            o_scr[pl.ds(g - 1, 1), :] = jnp.sum(o, axis=0, keepdims=True)

        @pl.when(g == 0)
        def _():
            q = q_scr[...]
            n = kfirst.shape[0] * _RB
            _wait_all(kfirst.at[pl.ds(0, KS // _RB)], wsem.at[6])
            if KS % _RB:
                _wait_all(kfirst.at[0, pl.ds(0, KS % _RB)], wsem.at[6])
            q0 = jnp.where((row == 0) & (col < KS), q, 0.0)[:_HG, :n].astype(bf16)
            carry_scr[...] = _dot(q0, kfirst[...].reshape(n, Sk))
            q = pltpu.roll(q, P - KS, 1)
            q_scr[...] = jnp.where(col < P - KS, q, pltpu.roll(q, n_groups - 1, 0))

        @pl.when(g < n_groups)
        def _():
            wait_rows(0, BR)
            wait_rows(1, BR)
            qd_scr[...] = jnp.where(k_diag, q_scr[pl.ds(g, 1), :], 0.0).astype(bf16)

            def scores_start(i):
                issue_cache(g, (4, 5), i)
                if cfg["compute"]:
                    cols = _tile(i, Sk // NS)
                    s_scr[:, cols] = _dot(qd_scr[:, :BR], block(0, cols)) + _dot(
                        qd_scr[:, BR:2 * BR], block(1, cols)
                    )

            _loop(0, NS, scores_start)

    _loop(0, n_groups + 1, group)

    down = list(down_copies())

    def issue_down(i):
        for cp, queue in down[len(down) * i // n_hg:len(down) * (i + 1) // n_hg]:
            cp.start(priority=queue)

    issue_down(0)
    _wait_all(vlast.at[pl.ds(0, VS)], wsem.at[7])
    o_last = (_dot_nt(p_scr[...], vlast[...]) / l_scr[...])[_HG - 1:_HG]
    o_last = jnp.concatenate([o_last, o_last], axis=1)
    o_last = jnp.concatenate([o_last] * (P // (2 * _RB)), axis=1)
    o = pltpu.roll(o_scr[...], P - VS, 1)
    o_next = jnp.where(row == n_groups - 1, o_last, pltpu.roll(o, n_groups - 1, 0))
    o_scr[...] = jnp.where(col < P - VS, o, o_next)

    _wait_all(wobuf, wsem.at[1])
    h_scr[...] = x
    n = wobuf.shape[0] // n_hg
    for i in range(n_hg):
        o = jnp.concatenate([o_scr[pl.ds(b % B * n_hg + i, 1), :] for b in range(2 * B)], axis=0)
        h_scr[...] += _dot(o.astype(bf16), wobuf[i * n:(i + 1) * n].reshape(P, D))
        if i + 1 < n_hg:
            issue_down(i + 1)

    h = h_scr[...]
    hn = _layernorm(h)
    hb = hn.astype(bf16)
    wr_cp.wait()
    r = jnp.sum(hn * wrbuf[...].astype(jnp.float32).reshape(1, D), axis=-1, keepdims=True)
    route = jax.nn.sigmoid(r)
    _wait_all(wgbuf, wsem.at[2])
    _wait_all(wubuf, wsem.at[3])
    gate = _dot(hb, wgbuf[...].reshape(D, F))
    up = _dot(hb, wubuf[...].reshape(D, F))
    act = (gate * jax.nn.sigmoid(gate) * up).astype(bf16)
    y = jnp.zeros((2 * B, D), jnp.float32)
    lo = 0
    for f, n in enumerate(cfg["wd"]):
        _wait_all(wdbuf.at[pl.ds(lo, n)], dsem.at[f])
        y = y + _dot(act[:, lo:lo + n], wdbuf[lo:lo + n])
        lo += n
    out = h + (hn + (hn * 0.0 + y * route))
    out_ref[...] = out[:B].astype(out_ref.dtype)


def build(**kw):
    cfg = dict(CFG, **kw)

    def kernel(A_x, A_k_cache, A_v_cache, A_wq, A_wo, B_x, B_w_r, B_w_gate, B_w_up, B_w_down):
        del B_x
        B, Sq, D = A_x.shape
        _, H, Sk, Dh = A_k_cache.shape
        F = B_w_gate.shape[1]
        P = _HG * Dh
        assert Sq == 1 and B * H == 2 * _HG * _HG and P == 3 * _NB * _RB
        assert _RB <= cfg["ks"] <= Dh and 0 < cfg["vs"] <= _RB
        dt = A_k_cache.dtype
        f32 = jnp.float32
        kt = jnp.swapaxes(A_k_cache, 2, 3).reshape(-1, _RB, Sk)
        vt = jnp.swapaxes(A_v_cache, 2, 3).reshape(-1, _RB, Sk)
        wq = A_wq.reshape(2 * cfg["wq"][0], -1, H * Dh)
        wo = A_wo.reshape(2 * cfg["wo"][0], -1, D)
        wg = B_w_gate.reshape(cfg["gu"][0], -1, F)
        wu = B_w_up.reshape(cfg["gu"][0], -1, F)
        out = pl.pallas_call(
            functools.partial(_body, B=B, H=H, Dh=Dh, Sk=Sk, D=D, F=F, cfg=cfg),
            in_specs=[pl.BlockSpec(memory_space=pl.ANY)] * 9,
            out_specs=pl.BlockSpec(memory_space=pltpu.VMEM),
            out_shape=jax.ShapeDtypeStruct((B, D), A_x.dtype),
            scratch_shapes=[
                pltpu.VMEM((6, _NB, _RB, Sk), dt),
                pltpu.VMEM((Dh // _RB, _RB, Sk), dt),
                pltpu.VMEM((_RB, Sk), dt),
                pltpu.VMEM(wq.shape, dt),
                pltpu.VMEM(wo.shape, dt),
                pltpu.VMEM(wg.shape, dt),
                pltpu.VMEM(wu.shape, dt),
                pltpu.VMEM(B_w_down.shape, dt),
                pltpu.VMEM((B, D), dt),
                pltpu.VMEM((D,), dt),
                pltpu.VMEM((2 * _HG, P), f32),
                pltpu.VMEM((2 * _HG, P), jnp.bfloat16),
                pltpu.VMEM((2 * _HG, Sk), f32),
                pltpu.VMEM((_HG, Sk), f32),
                pltpu.VMEM((2 * _HG, Sk), jnp.bfloat16),
                pltpu.VMEM((2 * _HG, 1), f32),
                pltpu.VMEM((2 * _HG, P), f32),
                pltpu.VMEM((2 * _HG, P), f32),
                pltpu.VMEM((2 * B, D), f32),
                pltpu.SemaphoreType.DMA((6,)),
                pltpu.SemaphoreType.DMA((8,)),
                pltpu.SemaphoreType.DMA((len(cfg["wd"]),)),
            ],
            compiler_params=pltpu.CompilerParams(
                vmem_limit_bytes=100 * 1024 * 1024, disable_bounds_checks=cfg["nb"]
            ),
        )(A_x.reshape(B, D), kt, vt, wq, wo, B_w_r, wg, wu, B_w_down)
        return out.reshape(B, Sq, D)

    return jax.jit(kernel)


pallas_sequential_preLN__mha_block_cached__moe_arch_mod__decode_kernel = build()
```

```python
import functools

import jax
import jax.numpy as jnp
import jax.experimental.pallas as pl
import jax.experimental.pallas.tpu as pltpu

_EPS = 1e-5
_HG = 8
_RB = 64
_NB = 8
_CW = 1024
CFG = dict(compute=True, wq=(5, 384), wo=(4, 640), gu=(4, 512), wd=(768, 512, 256), dr=32, nb=True, ks=176, vs=40, o0=(0, 2, 4, 6), o1=(0, 2, 4, 6), pw=1024)


def _layernorm(x):
    m = jnp.mean(x, axis=-1, keepdims=True)
    d = x - m
    v = jnp.mean(d * d, axis=-1, keepdims=True)
    return d / jnp.sqrt(v + _EPS)


def _dot(a, b):
    return jnp.dot(a, b, preferred_element_type=jnp.float32)


def _dot_nt(a, b):
    return jax.lax.dot_general(
        a, b, (((1,), (1,)), ((), ())), preferred_element_type=jnp.float32
    )


def _wait_all(buf, sem):
    pltpu.make_async_copy(buf, buf, sem).wait()


def _loop(lo, hi, fn):
    jax.lax.fori_loop(lo, hi, lambda i, carry: fn(i), None)


def _tile(i, n):
    return pl.ds(i * n if isinstance(i, int) else pl.multiple_of(i * n, n), n)


def _body(
    x_hbm, kt_hbm, vt_hbm, wq_hbm, wo_hbm, wr_hbm, wg_hbm, wu_hbm, wd_hbm,
    out_ref,
    cbuf, kfirst, vlast, wqbuf, wobuf, wgbuf, wubuf, wdbuf, xbuf, wrbuf,
    q_scr, qd_scr, s_scr, carry_scr, p_scr, l_scr, acc_scr, o_scr, h_scr,
    csem, wsem, dsem,
    *, B, H, Dh, Sk, D, F, cfg,
):
    P = _HG * Dh
    BR = _NB * _RB
    NS = _RB // 8
    n_hg = H // _HG
    n_groups = B * n_hg
    n_bands = kt_hbm.shape[0]
    scale = Dh ** -0.5
    bf16 = jnp.bfloat16
    KS, VS = cfg["ks"], cfg["vs"]

    def cache_copy(g, blk, i, cols, lo, hi):
        src, r = (kt_hbm, 8 * i + KS) if blk < 3 else (vt_hbm, 8 * i + _RB * _NB - VS)
        band = (g * 3 + blk % 3) * _NB + r // _RB - (0 if blk < 3 else _NB)
        return pltpu.make_async_copy(
            src.at[pl.ds(band + lo, hi - lo), _tile(r % _RB // 8, 8), cols],
            cbuf.at[blk, pl.ds(lo, hi - lo), _tile(i, 8), cols],
            csem.at[blk],
        )

    def issue_cache(g, blocks, i):
        for c in range(Sk // _CW):
            for bands in zip(cfg["o0"], cfg["o1"]):
                for queue, blk in enumerate(blocks):
                    n = bands[queue]
                    cache_copy(g, blk, i, _tile(c, _CW), n, n + 2).start(priority=queue)

    def issue_edge(g, i):
        limits = [
            (-((8 * j - VS) // _RB) if g == 0 else 0, _NB - (8 * j + KS) // _RB if g else _NB)
            for j in range(NS)
        ]
        for lo, hi in sorted(set(limits)):
            steps = [j for j in range(NS) if limits[j] == (lo, hi)]

            @pl.when((i >= steps[0]) & (i <= steps[-1]))
            def _(lo=lo, hi=hi):
                def piece(c):
                    cols = _tile(c, _CW)
                    for n, m in zip(cfg["o0"], cfg["o1"]):
                        if n < hi:
                            cache_copy(g, 2, i, cols, n, min(n + 2, hi)).start(priority=0)
                        cache_copy(g, 3, i, cols, max(m, lo), m + 2).start(priority=1)

                _loop(0, Sk // _CW, piece)

    def wait_rows(blk, n):
        _wait_all(cbuf.at[blk, pl.ds(0, n // _RB)], csem.at[blk])
        if n % _RB:
            _wait_all(cbuf.at[blk, 0, pl.ds(0, n % _RB)], csem.at[blk])

    def issue_k_first():
        for r in range(0, _RB, 8):
            n = -((r - KS) // _RB)

            def piece(c, r=r, n=n):
                for queue in range(2):
                    idx = (pl.ds(0, n), pl.ds(r, 8), _tile(c + queue * (Sk // cfg["pw"] // 2), cfg["pw"]))
                    pltpu.make_async_copy(kt_hbm.at[idx], kfirst.at[idx], wsem.at[6]).start(priority=queue)

            if n > 0:
                _loop(0, Sk // cfg["pw"] // 2, piece)

    def issue_v_last():
        def piece(c):
            for queue in range(2):
                rows, cols = pl.ds(_RB - VS, VS), _tile(c + queue * (Sk // 1024), 512)
                pltpu.make_async_copy(
                    vt_hbm.at[n_bands - 1, rows, cols], vlast.at[rows, cols], wsem.at[7]
                ).start(priority=queue)

        _loop(0, Sk // 1024, piece)

    def issue_halves(src, dst, sem, cw, i):
        n = src.shape[0] // 2
        for c in range(0, src.shape[2], cw):
            for queue in range(2):
                idx = (pl.ds(queue * n, n), _tile(i, 8), pl.ds(c, min(cw, src.shape[2] - c)))
                pltpu.make_async_copy(src.at[idx], dst.at[idx], sem).start(priority=queue)

    def issue_gate_up(i):
        cw = cfg["gu"][1]
        for c in range(0, F, cw):
            idx = (slice(None), _tile(i, 8), pl.ds(c, cw))
            pltpu.make_async_copy(wg_hbm.at[idx], wgbuf.at[idx], wsem.at[2]).start(priority=0)
            pltpu.make_async_copy(wu_hbm.at[idx], wubuf.at[idx], wsem.at[3]).start(priority=1)

    def down_copies():
        lo = 0
        for f, n in enumerate(cfg["wd"]):
            dr = cfg["dr"]
            for i in range(n // dr):
                rows = pl.ds(lo + (i % 2) * (n // 2) + (i // 2) * dr, dr)
                yield pltpu.make_async_copy(wd_hbm.at[rows, :], wdbuf.at[rows, :], dsem.at[f]), i % 2
            lo += n

    x_cp = pltpu.make_async_copy(x_hbm, xbuf, wsem.at[4])
    wr_cp = pltpu.make_async_copy(wr_hbm, wrbuf, wsem.at[5])
    issue_wq = functools.partial(issue_halves, wq_hbm, wqbuf, wsem.at[0], cfg["wq"][1])
    _loop(0, 2, issue_wq)
    x_cp.start()
    wr_cp.start(priority=1)
    kfirst[...] = jnp.zeros_like(kfirst)
    vlast[...] = jnp.zeros_like(vlast)
    cbuf[3, 0] = jnp.zeros((_RB, Sk), cbuf.dtype)
    _loop(2, wq_hbm.shape[1] // 8, issue_wq)
    issue_k_first()

    x_cp.wait()
    x4 = xbuf[...].astype(jnp.float32)
    x = jnp.concatenate([x4, x4], axis=0)
    xn = _layernorm(x).astype(bf16)
    row = jax.lax.broadcasted_iota(jnp.int32, (2 * _HG, P), 0)
    col = jax.lax.broadcasted_iota(jnp.int32, (2 * _HG, P), 1)
    k_diag = (col + KS >= row * Dh) & (col + KS < row * Dh + Dh)
    v_row = jnp.where(row < _HG, row, row - 2 * _HG)
    v_diag = (col - VS >= v_row * Dh) & (col - VS < v_row * Dh + Dh)
    p_scr[...] = jnp.zeros_like(p_scr)
    l_scr[...] = jnp.ones_like(l_scr)

    def block(blk, cols):
        return cbuf[blk, :, :, cols].reshape(BR, cols.size)

    n_wo = wo_hbm.shape[1] // 8
    n_gu = wg_hbm.shape[1] // 8
    T_WO = 11

    def issue_tail(t):
        u = jnp.maximum(t - T_WO, 0)
        v = jnp.maximum(t + 1 - T_WO, 0)
        _loop(
            jnp.minimum(t, T_WO) * n_wo // T_WO,
            jnp.minimum(t + 1, T_WO) * n_wo // T_WO,
            functools.partial(issue_halves, wo_hbm, wobuf, wsem.at[1], cfg["wo"][1]),
        )
        _loop(u * n_gu // (2 * NS - T_WO), v * n_gu // (2 * NS - T_WO), issue_gate_up)

    def group(g):
        started = (g > 0) & cfg["compute"]

        @pl.when((g > 0) & (g < n_groups))
        def _():
            wait_rows(2, BR)

        @pl.when(g == n_groups)
        def _():
            issue_v_last()
            wait_rows(2, BR - KS)

        pl.when(g > 1)(lambda: wait_rows(3, BR))
        pl.when(g == 1)(lambda: wait_rows(3, BR - VS))

        def issue_first(i):
            pl.when(g < n_groups)(lambda: issue_cache(g, (0, 1), i))
            pl.when(g == n_groups)(lambda: issue_tail(i))

        def scores_end(i):
            issue_first(i)

            @pl.when(started)
            def _():
                cols = _tile(i, 2 * Sk // NS)
                s_scr[:, cols] += _dot(qd_scr[:, 2 * BR:], block(2, cols))

        _loop(0, NS // 2, scores_end)

        @pl.when(started)
        def _():
            s = (s_scr[:_HG] + carry_scr[...]) * scale
            carry_scr[...] = s_scr[_HG:]
            e = jnp.exp(s - jnp.max(s, axis=-1, keepdims=True))
            e_prev = p_scr[...].astype(jnp.float32)[:_HG]
            p_scr[...] = jnp.concatenate([e, e_prev], axis=0).astype(bf16)
            l_scr[_HG:] = l_scr[:_HG]
            l_scr[:_HG] = jnp.sum(e, axis=-1, keepdims=True)
            acc_scr[...] = jnp.zeros_like(acc_scr)

        def values_start(i):
            issue_first(NS // 2 + i)

            @pl.when(started)
            def _():
                cols = _tile(i, 2 * Sk // NS)
                acc_scr[:, :BR] += _dot_nt(p_scr[:, cols], block(3, cols))

        _loop(0, NS // 2, values_start)

        @pl.when(g > 0)
        def _():
            wait_rows(4, BR)
            wait_rows(5, BR)

        @pl.when(g == 0)
        def _():
            _wait_all(wqbuf, wsem.at[0])

        @pl.when(g == n_groups - 1)
        def _():
            n = -(-KS // _RB)
            cbuf[2, _NB - n:] = jnp.zeros((n, _RB, Sk), cbuf.dtype)

        def values_end(i):
            pl.when((g > 0) & (g < n_groups - 1))(lambda: issue_cache(g, (2, 3), i))
            pl.when(g == 0)(lambda: issue_edge(0, i))
            pl.when(g == n_groups - 1)(lambda: issue_edge(n_groups - 1, i))
            pl.when(g == n_groups)(lambda: issue_tail(NS + i))

            @pl.when(started)
            def _():
                cols = _tile(i, Sk // NS)
                p = p_scr[:, cols]
                acc_scr[:, BR:2 * BR] += _dot_nt(p, block(4, cols))
                acc_scr[:, 2 * BR:] += _dot_nt(p, block(5, cols))

            @pl.when((g == 0) & (i < n_hg))
            def _():
                q = _dot(xn, wqbuf[:, :, _tile(i, P)].reshape(D, P))
                for b in range(B):
                    q_scr[pl.ds(b * n_hg + i, 1), :] = q[b:b + 1]

        _loop(0, NS, values_end)

        @pl.when(started)
        def _():
            o = jnp.where(v_diag, acc_scr[...] / l_scr[...], 0.0)
            o_scr[pl.ds(g - 1, 1), :] = jnp.sum(o, axis=0, keepdims=True)

        @pl.when(g == 0)
        def _():
            q = q_scr[...]
            n = kfirst.shape[0] * _RB
            _wait_all(kfirst.at[pl.ds(0, KS // _RB)], wsem.at[6])
            if KS % _RB:
                _wait_all(kfirst.at[0, pl.ds(0, KS % _RB)], wsem.at[6])
            q0 = jnp.where((row == 0) & (col < KS), q, 0.0)[:_HG, :n].astype(bf16)
            carry_scr[...] = _dot(q0, kfirst[...].reshape(n, Sk))
            q = pltpu.roll(q, P - KS, 1)
            q_scr[...] = jnp.where(col < P - KS, q, pltpu.roll(q, n_groups - 1, 0))

        @pl.when(g < n_groups)
        def _():
            wait_rows(0, BR)
            wait_rows(1, BR)
            qd_scr[...] = jnp.where(k_diag, q_scr[pl.ds(g, 1), :], 0.0).astype(bf16)

            def scores_start(i):
                issue_cache(g, (4, 5), i)
                if cfg["compute"]:
                    cols = _tile(i, Sk // NS)
                    s_scr[:, cols] = _dot(qd_scr[:, :BR], block(0, cols)) + _dot(
                        qd_scr[:, BR:2 * BR], block(1, cols)
                    )

            _loop(0, NS, scores_start)

    _loop(0, n_groups + 1, group)

    down = list(down_copies())

    def issue_down(i):
        for cp, queue in down[len(down) * i // n_hg:len(down) * (i + 1) // n_hg]:
            cp.start(priority=queue)

    issue_down(0)
    _wait_all(vlast.at[pl.ds(0, VS)], wsem.at[7])
    o_last = (_dot_nt(p_scr[...], vlast[...]) / l_scr[...])[_HG - 1:_HG]
    o_last = jnp.concatenate([o_last, o_last], axis=1)
    o_last = jnp.concatenate([o_last] * (P // (2 * _RB)), axis=1)
    o = pltpu.roll(o_scr[...], P - VS, 1)
    o_next = jnp.where(row == n_groups - 1, o_last, pltpu.roll(o, n_groups - 1, 0))
    o_scr[...] = jnp.where(col < P - VS, o, o_next)

    _wait_all(wobuf, wsem.at[1])
    h_scr[...] = x
    n = wobuf.shape[0] // n_hg
    for i in range(n_hg):
        o = jnp.concatenate([o_scr[pl.ds(b % B * n_hg + i, 1), :] for b in range(2 * B)], axis=0)
        h_scr[...] += _dot(o.astype(bf16), wobuf[i * n:(i + 1) * n].reshape(P, D))
        if i + 1 < n_hg:
            issue_down(i + 1)

    h = h_scr[...]
    hn = _layernorm(h)
    hb = hn.astype(bf16)
    wr_cp.wait()
    r = jnp.sum(hn * wrbuf[...].astype(jnp.float32).reshape(1, D), axis=-1, keepdims=True)
    route = jax.nn.sigmoid(r)
    _wait_all(wgbuf, wsem.at[2])
    _wait_all(wubuf, wsem.at[3])
    gate = _dot(hb, wgbuf[...].reshape(D, F))
    up = _dot(hb, wubuf[...].reshape(D, F))
    act = (gate * jax.nn.sigmoid(gate) * up).astype(bf16)
    y = jnp.zeros((2 * B, D), jnp.float32)
    lo = 0
    for f, n in enumerate(cfg["wd"]):
        _wait_all(wdbuf.at[pl.ds(lo, n)], dsem.at[f])
        y = y + _dot(act[:, lo:lo + n], wdbuf[lo:lo + n])
        lo += n
    out = h + (hn + (hn * 0.0 + y * route))
    out_ref[...] = out[:B].astype(out_ref.dtype)


def build(**kw):
    cfg = dict(CFG, **kw)

    def kernel(A_x, A_k_cache, A_v_cache, A_wq, A_wo, B_x, B_w_r, B_w_gate, B_w_up, B_w_down):
        del B_x
        B, Sq, D = A_x.shape
        _, H, Sk, Dh = A_k_cache.shape
        F = B_w_gate.shape[1]
        P = _HG * Dh
        assert Sq == 1 and B * H == 2 * _HG * _HG and P == 3 * _NB * _RB
        assert _RB <= cfg["ks"] <= Dh and 0 < cfg["vs"] <= _RB
        dt = A_k_cache.dtype
        f32 = jnp.float32
        kt = jnp.swapaxes(A_k_cache, 2, 3).reshape(-1, _RB, Sk)
        vt = jnp.swapaxes(A_v_cache, 2, 3).reshape(-1, _RB, Sk)
        wq = A_wq.reshape(2 * cfg["wq"][0], -1, H * Dh)
        wo = A_wo.reshape(2 * cfg["wo"][0], -1, D)
        wg = B_w_gate.reshape(cfg["gu"][0], -1, F)
        wu = B_w_up.reshape(cfg["gu"][0], -1, F)
        out = pl.pallas_call(
            functools.partial(_body, B=B, H=H, Dh=Dh, Sk=Sk, D=D, F=F, cfg=cfg),
            in_specs=[pl.BlockSpec(memory_space=pl.ANY)] * 9,
            out_specs=pl.BlockSpec(memory_space=pltpu.VMEM),
            out_shape=jax.ShapeDtypeStruct((B, D), A_x.dtype),
            scratch_shapes=[
                pltpu.VMEM((6, _NB, _RB, Sk), dt),
                pltpu.VMEM((Dh // _RB, _RB, Sk), dt),
                pltpu.VMEM((_RB, Sk), dt),
                pltpu.VMEM(wq.shape, dt),
                pltpu.VMEM(wo.shape, dt),
                pltpu.VMEM(wg.shape, dt),
                pltpu.VMEM(wu.shape, dt),
                pltpu.VMEM(B_w_down.shape, dt),
                pltpu.VMEM((B, D), dt),
                pltpu.VMEM((D,), dt),
                pltpu.VMEM((2 * _HG, P), f32),
                pltpu.VMEM((2 * _HG, P), jnp.bfloat16),
                pltpu.VMEM((2 * _HG, Sk), f32),
                pltpu.VMEM((_HG, Sk), f32),
                pltpu.VMEM((2 * _HG, Sk), jnp.bfloat16),
                pltpu.VMEM((2 * _HG, 1), f32),
                pltpu.VMEM((2 * _HG, P), f32),
                pltpu.VMEM((2 * _HG, P), f32),
                pltpu.VMEM((2 * B, D), f32),
                pltpu.SemaphoreType.DMA((6,)),
                pltpu.SemaphoreType.DMA((8,)),
                pltpu.SemaphoreType.DMA((len(cfg["wd"]),)),
            ],
            compiler_params=pltpu.CompilerParams(
                vmem_limit_bytes=100 * 1024 * 1024, disable_bounds_checks=cfg["nb"]
            ),
        )(A_x.reshape(B, D), kt, vt, wq, wo, B_w_r, wg, wu, B_w_down)
        return out.reshape(B, Sq, D)

    return jax.jit(kernel)


pallas_sequential_preLN__mha_block_cached__moe_arch_mod__decode_kernel = build()
```

```python
import functools

import jax
import jax.numpy as jnp
import jax.experimental.pallas as pl
import jax.experimental.pallas.tpu as pltpu

_EPS = 1e-5
_HG = 8
_RB = 64
_NB = 8
_CW = 1024
_K_SHIFT = 176
_V_SHIFT = 40
_WQ_BANDS, _WQ_CW = 10, 384
_WO_BANDS = 8
_GU_BANDS, _GU_CW = 4, 512
_WD_ROWS = 24
_WO_STEPS = 11


def _layernorm(x):
    m = jnp.mean(x, axis=-1, keepdims=True)
    d = x - m
    v = jnp.mean(d * d, axis=-1, keepdims=True)
    return d / jnp.sqrt(v + _EPS)


def _dot(a, b):
    return jnp.dot(a, b, preferred_element_type=jnp.float32)


def _dot_nt(a, b):
    return jax.lax.dot_general(
        a, b, (((1,), (1,)), ((), ())), preferred_element_type=jnp.float32
    )


def _wait_all(buf, sem):
    pltpu.make_async_copy(buf, buf, sem).wait()


def _wait_rows(buf, sem, n):
    _wait_all(buf.at[pl.ds(0, n // _RB)], sem)
    if n % _RB:
        _wait_all(buf.at[n // _RB, pl.ds(0, n % _RB)], sem)


def _loop(lo, hi, fn):
    jax.lax.fori_loop(lo, hi, lambda i, carry: fn(i), None)


def _tile(i, n):
    return pl.ds(i * n if isinstance(i, int) else pl.multiple_of(i * n, n), n)


def _body(
    x_hbm, kt_hbm, vt_hbm, wq_hbm, wo_hbm, wr_hbm, wg_hbm, wu_hbm, wd_hbm,
    out_ref,
    cbuf, kfirst, vlast, wqbuf, wobuf, wgbuf, wubuf, wdbuf, xbuf, wrbuf,
    q_scr, qd_scr, s_scr, carry_scr, p_scr, l_scr, acc_scr, o_scr, h_scr,
    csem, dsem, ksem, vsem, wqsem, wosem, wgsem, wusem, xsem, wrsem,
    *, B, H, Dh, Sk, D, F,
):
    P = _HG * Dh
    BR = _NB * _RB
    NS = _RB // 8
    NC = Sk // _CW
    n_hg = H // _HG
    n_groups = B * n_hg
    scale = Dh ** -0.5
    bf16 = jnp.bfloat16

    def cache_copy(g, blk, i, cols, lo, hi):
        band = (g * 3 + blk % 3) * _NB
        if blk < 3:
            src, r = kt_hbm, 8 * i + _K_SHIFT
        else:
            src, r, band = vt_hbm, 8 * i + _RB - _V_SHIFT, band - 1
        return pltpu.make_async_copy(
            src.at[pl.ds(band + r // _RB + lo, hi - lo), _tile(r % _RB // 8, 8), cols],
            cbuf.at[blk, pl.ds(lo, hi - lo), _tile(i, 8), cols],
            csem.at[blk],
        )

    def issue_cache(g, blocks, i):
        for c in range(NC):
            for n in range(0, _NB, 2):
                for queue, blk in enumerate(blocks):
                    cache_copy(g, blk, i, _tile(c, _CW), n, n + 2).start(priority=queue)

    def issue_edge(g, i):
        if g == 0:
            limits = [(int(8 * j < _V_SHIFT), _NB) for j in range(NS)]
        else:
            limits = [(0, _NB - (8 * j + _K_SHIFT) // _RB) for j in range(NS)]
        for lo, hi in sorted(set(limits)):
            steps = [j for j in range(NS) if limits[j] == (lo, hi)]

            def piece(c, lo=lo, hi=hi):
                cols = _tile(c, _CW)
                for n in range(0, _NB, 2):
                    if n < hi:
                        cache_copy(g, 2, i, cols, n, min(n + 2, hi)).start(priority=0)
                    cache_copy(g, 3, i, cols, max(n, lo), n + 2).start(priority=1)

            pl.when((i >= steps[0]) & (i <= steps[-1]))(functools.partial(_loop, 0, NC, piece))

    def issue_k_first():
        for r in range(0, _RB, 8):

            def piece(c, r=r):
                for queue in range(2):
                    bands = pl.ds(0, pl.cdiv(_K_SHIFT - r, _RB))
                    idx = (bands, pl.ds(r, 8), _tile(c + queue * (NC // 2), _CW))
                    pltpu.make_async_copy(kt_hbm.at[idx], kfirst.at[idx], ksem).start(
                        priority=queue
                    )

            _loop(0, NC // 2, piece)

    def issue_v_last():
        def piece(c):
            for queue in range(2):
                rows, cols = pl.ds(_RB - _V_SHIFT, _V_SHIFT), _tile(c + queue * NC, _CW // 2)
                pltpu.make_async_copy(
                    vt_hbm.at[vt_hbm.shape[0] - 1, rows, cols], vlast.at[rows, cols], vsem
                ).start(priority=queue)

        _loop(0, NC, piece)

    def issue_halves(src, dst, sem, cw, i):
        n = src.shape[0] // 2
        for c in range(0, src.shape[2], cw):
            for queue in range(2):
                idx = (pl.ds(queue * n, n), _tile(i, 8), pl.ds(c, cw))
                pltpu.make_async_copy(src.at[idx], dst.at[idx], sem).start(priority=queue)

    def issue_gate_up(i):
        for c in range(0, F, _GU_CW):
            idx = (slice(None), _tile(i, 8), pl.ds(c, _GU_CW))
            pltpu.make_async_copy(wg_hbm.at[idx], wgbuf.at[idx], wgsem).start(priority=0)
            pltpu.make_async_copy(wu_hbm.at[idx], wubuf.at[idx], wusem).start(priority=1)

    def issue_weights(t):
        n_wo, n_gu, rest = wobuf.shape[1] // 8, wgbuf.shape[1] // 8, 2 * NS - _WO_STEPS
        _loop(
            jnp.minimum(t, _WO_STEPS) * n_wo // _WO_STEPS,
            jnp.minimum(t + 1, _WO_STEPS) * n_wo // _WO_STEPS,
            functools.partial(issue_halves, wo_hbm, wobuf, wosem, D),
        )
        _loop(
            jnp.maximum(t - _WO_STEPS, 0) * n_gu // rest,
            jnp.maximum(t + 1 - _WO_STEPS, 0) * n_gu // rest,
            issue_gate_up,
        )

    def issue_down(f):
        half = wdbuf.shape[1] // 2
        for r in range(0, half, _WD_ROWS):
            for queue in range(2):
                idx = (f, pl.ds(queue * half + r, _WD_ROWS))
                pltpu.make_async_copy(wd_hbm.at[idx], wdbuf.at[idx], dsem.at[f]).start(
                    priority=queue
                )

    x_cp = pltpu.make_async_copy(x_hbm, xbuf, xsem)
    wr_cp = pltpu.make_async_copy(wr_hbm, wrbuf, wrsem)
    issue_wq = functools.partial(issue_halves, wq_hbm, wqbuf, wqsem, _WQ_CW)
    _loop(0, 2, issue_wq)
    x_cp.start()
    wr_cp.start(priority=1)
    kfirst[...] = jnp.zeros_like(kfirst)
    vlast[...] = jnp.zeros_like(vlast)
    cbuf[3, 0] = jnp.zeros((_RB, Sk), cbuf.dtype)
    _loop(2, wqbuf.shape[1] // 8, issue_wq)
    issue_k_first()

    x_cp.wait()
    x = xbuf[...].astype(jnp.float32)
    x = jnp.concatenate([x, x], axis=0)
    xn = _layernorm(x).astype(bf16)
    row = jax.lax.broadcasted_iota(jnp.int32, (2 * _HG, P), 0)
    col = jax.lax.broadcasted_iota(jnp.int32, (2 * _HG, P), 1)
    k_diag = (col + _K_SHIFT >= row * Dh) & (col + _K_SHIFT < row * Dh + Dh)
    v_row = jnp.where(row < _HG, row, row - 2 * _HG)
    v_diag = (col - _V_SHIFT >= v_row * Dh) & (col - _V_SHIFT < v_row * Dh + Dh)
    p_scr[...] = jnp.zeros_like(p_scr)
    l_scr[...] = jnp.ones_like(l_scr)

    def block(blk, cols):
        return cbuf[blk, :, :, cols].reshape(BR, cols.size)

    def wait_block(blk):
        _wait_all(cbuf.at[blk], csem.at[blk])

    def group(g):
        pl.when((g > 0) & (g < n_groups))(lambda: wait_block(2))
        pl.when(g > 1)(lambda: wait_block(3))

        @pl.when(g == 1)
        def _():
            _wait_all(cbuf.at[3, pl.ds(1, _NB - 1)], csem.at[3])
            _wait_all(cbuf.at[3, 0, pl.ds(_V_SHIFT, _RB - _V_SHIFT)], csem.at[3])

        @pl.when(g == n_groups)
        def _():
            issue_v_last()
            _wait_rows(cbuf.at[2], csem.at[2], BR - _K_SHIFT)

        def issue_first(i):
            pl.when(g < n_groups)(lambda: issue_cache(g, (0, 1), i))
            pl.when(g == n_groups)(lambda: issue_weights(i))

        def scores_end(i):
            issue_first(i)

            @pl.when(g > 0)
            def _():
                cols = _tile(i, 2 * Sk // NS)
                s_scr[:, cols] += _dot(qd_scr[:, 2 * BR:], block(2, cols))

        _loop(0, NS // 2, scores_end)

        @pl.when(g > 0)
        def _():
            s = (s_scr[:_HG] + carry_scr[...]) * scale
            carry_scr[...] = s_scr[_HG:]
            e = jnp.exp(s - jnp.max(s, axis=-1, keepdims=True))
            e_prev = p_scr[...].astype(jnp.float32)[:_HG]
            p_scr[...] = jnp.concatenate([e, e_prev], axis=0).astype(bf16)
            l_scr[_HG:] = l_scr[:_HG]
            l_scr[:_HG] = jnp.sum(e, axis=-1, keepdims=True)
            acc_scr[...] = jnp.zeros_like(acc_scr)

        def values_start(i):
            issue_first(NS // 2 + i)

            @pl.when(g > 0)
            def _():
                cols = _tile(i, 2 * Sk // NS)
                acc_scr[:, :BR] += _dot_nt(p_scr[:, cols], block(3, cols))

        _loop(0, NS // 2, values_start)

        @pl.when(g > 0)
        def _():
            wait_block(4)
            wait_block(5)

        pl.when(g == 0)(lambda: _wait_all(wqbuf, wqsem))

        @pl.when(g == n_groups - 1)
        def _():
            n = pl.cdiv(_K_SHIFT, _RB)
            cbuf[2, _NB - n:] = jnp.zeros((n, _RB, Sk), cbuf.dtype)

        def values_end(i):
            pl.when((g > 0) & (g < n_groups - 1))(lambda: issue_cache(g, (2, 3), i))
            pl.when(g == 0)(lambda: issue_edge(0, i))
            pl.when(g == n_groups - 1)(lambda: issue_edge(n_groups - 1, i))
            pl.when(g == n_groups)(lambda: issue_weights(NS + i))

            @pl.when(g > 0)
            def _():
                cols = _tile(i, Sk // NS)
                p = p_scr[:, cols]
                acc_scr[:, BR:2 * BR] += _dot_nt(p, block(4, cols))
                acc_scr[:, 2 * BR:] += _dot_nt(p, block(5, cols))

            @pl.when((g == 0) & (i < n_hg))
            def _():
                q = _dot(xn, wqbuf[:, :, _tile(i, P)].reshape(D, P))
                for b in range(B):
                    q_scr[pl.ds(b * n_hg + i, 1), :] = q[b:b + 1]

        _loop(0, NS, values_end)

        @pl.when(g > 0)
        def _():
            o = jnp.where(v_diag, acc_scr[...] / l_scr[...], 0.0)
            o_scr[pl.ds(g - 1, 1), :] = jnp.sum(o, axis=0, keepdims=True)

        @pl.when(g == 0)
        def _():
            q = q_scr[...]
            _wait_rows(kfirst, ksem, _K_SHIFT)
            q0 = jnp.where((row == 0) & (col < _K_SHIFT), q, 0.0)[:_HG, :Dh].astype(bf16)
            carry_scr[...] = _dot(q0, kfirst[...].reshape(Dh, Sk))
            q = pltpu.roll(q, P - _K_SHIFT, 1)
            q_scr[...] = jnp.where(col < P - _K_SHIFT, q, pltpu.roll(q, n_groups - 1, 0))

        @pl.when(g < n_groups)
        def _():
            wait_block(0)
            wait_block(1)
            qd_scr[...] = jnp.where(k_diag, q_scr[pl.ds(g, 1), :], 0.0).astype(bf16)

            def scores_start(i):
                issue_cache(g, (4, 5), i)
                cols = _tile(i, Sk // NS)
                s_scr[:, cols] = _dot(qd_scr[:, :BR], block(0, cols)) + _dot(
                    qd_scr[:, BR:2 * BR], block(1, cols)
                )

            _loop(0, NS, scores_start)

    _loop(0, n_groups + 1, group)

    issue_down(0)
    _wait_all(vlast.at[pl.ds(_RB - _V_SHIFT, _V_SHIFT)], vsem)
    o_last = (_dot_nt(p_scr[...], vlast[...]) / l_scr[...])[_HG - 1:_HG]
    o_last = jnp.concatenate([o_last, o_last], axis=1)
    o_last = jnp.concatenate([o_last] * (P // (2 * _RB)), axis=1)
    o = pltpu.roll(o_scr[...], P - _V_SHIFT, 1)
    o_next = jnp.where(row == n_groups - 1, o_last, pltpu.roll(o, n_groups - 1, 0))
    o_scr[...] = jnp.where(col < P - _V_SHIFT, o, o_next)

    _wait_all(wobuf, wosem)
    h_scr[...] = x
    n = _WO_BANDS // n_hg
    for i in range(n_hg):
        o = jnp.concatenate([o_scr[pl.ds(b % B * n_hg + i, 1), :] for b in range(2 * B)], axis=0)
        h_scr[...] += _dot(o.astype(bf16), wobuf[i * n:(i + 1) * n].reshape(P, D))
        if i + 1 < n_hg:
            issue_down(i + 1)

    h = h_scr[...]
    hn = _layernorm(h)
    hb = hn.astype(bf16)
    wr_cp.wait()
    r = jnp.sum(hn * wrbuf[...].astype(jnp.float32).reshape(1, D), axis=-1, keepdims=True)
    route = jax.nn.sigmoid(r)
    _wait_all(wgbuf, wgsem)
    _wait_all(wubuf, wusem)
    gate = _dot(hb, wgbuf[...].reshape(D, F))
    up = _dot(hb, wubuf[...].reshape(D, F))
    act = (gate * jax.nn.sigmoid(gate) * up).astype(bf16)
    y = jnp.zeros((2 * B, D), jnp.float32)
    n = F // n_hg
    for f in range(n_hg):
        _wait_all(wdbuf.at[f], dsem.at[f])
        y = y + _dot(act[:, f * n:(f + 1) * n], wdbuf[f])
    out = h + (hn + (hn * 0.0 + y * route))
    out_ref[...] = out[:B].astype(out_ref.dtype)


@jax.jit
def pallas_sequential_preLN__mha_block_cached__moe_arch_mod__decode_kernel(
    A_x: jax.Array,
    A_k_cache: jax.Array,
    A_v_cache: jax.Array,
    A_wq: jax.Array,
    A_wo: jax.Array,
    B_x: jax.Array,
    B_w_r: jax.Array,
    B_w_gate: jax.Array,
    B_w_up: jax.Array,
    B_w_down: jax.Array,
):
    del B_x
    B, Sq, D = A_x.shape
    _, H, Sk, Dh = A_k_cache.shape
    F = B_w_gate.shape[1]
    P = _HG * Dh
    n_hg = H // _HG
    assert Sq == 1 and B * n_hg == 2 * _HG and P == 3 * _NB * _RB and Sk % (2 * _CW) == 0
    assert _RB <= _K_SHIFT <= Dh and 0 < _V_SHIFT < _RB and F % (2 * n_hg * _WD_ROWS) == 0
    dt = A_k_cache.dtype
    f32 = jnp.float32

    kt = jnp.swapaxes(A_k_cache, 2, 3).reshape(-1, _RB, Sk)
    vt = jnp.swapaxes(A_v_cache, 2, 3).reshape(-1, _RB, Sk)
    wq = A_wq.reshape(_WQ_BANDS, -1, H * Dh)
    wo = A_wo.reshape(_WO_BANDS, -1, D)
    wg = B_w_gate.reshape(_GU_BANDS, -1, F)
    wu = B_w_up.reshape(_GU_BANDS, -1, F)
    wd = B_w_down.reshape(n_hg, -1, D)

    out = pl.pallas_call(
        functools.partial(_body, B=B, H=H, Dh=Dh, Sk=Sk, D=D, F=F),
        in_specs=[pl.BlockSpec(memory_space=pl.ANY)] * 9,
        out_specs=pl.BlockSpec(memory_space=pltpu.VMEM),
        out_shape=jax.ShapeDtypeStruct((B, D), A_x.dtype),
        scratch_shapes=[
            pltpu.VMEM((6, _NB, _RB, Sk), dt),
            pltpu.VMEM((Dh // _RB, _RB, Sk), dt),
            pltpu.VMEM((_RB, Sk), dt),
            *[pltpu.VMEM(w.shape, dt) for w in (wq, wo, wg, wu, wd)],
            pltpu.VMEM((B, D), dt),
            pltpu.VMEM((D,), dt),
            pltpu.VMEM((2 * _HG, P), f32),
            pltpu.VMEM((2 * _HG, P), jnp.bfloat16),
            pltpu.VMEM((2 * _HG, Sk), f32),
            pltpu.VMEM((_HG, Sk), f32),
            pltpu.VMEM((2 * _HG, Sk), jnp.bfloat16),
            pltpu.VMEM((2 * _HG, 1), f32),
            pltpu.VMEM((2 * _HG, P), f32),
            pltpu.VMEM((2 * _HG, P), f32),
            pltpu.VMEM((2 * B, D), f32),
            pltpu.SemaphoreType.DMA((6,)),
            pltpu.SemaphoreType.DMA((n_hg,)),
            *[pltpu.SemaphoreType.DMA(())] * 8,
        ],
        compiler_params=pltpu.CompilerParams(vmem_limit_bytes=100 * 1024 * 1024),
    )(A_x.reshape(B, D), kt, vt, wq, wo, B_w_r, wg, wu, wd)
    return out.reshape(B, Sq, D)
```

```python
import functools

import jax
import jax.numpy as jnp
import jax.experimental.pallas as pl
import jax.experimental.pallas.tpu as pltpu

_EPS = 1e-5
_HG = 8
_RB = 64
_NB = 8
_CW = 1024
_K_SHIFT = 176
_V_SHIFT = 40
_WQ_BANDS, _WQ_CW = 10, 384
_WO_BANDS = 8
_GU_BANDS, _GU_CW = 4, 512
_WD_ROWS = 24
_NS = 16
_WO_STEPS = 11


def _layernorm(x):
    m = jnp.mean(x, axis=-1, keepdims=True)
    d = x - m
    v = jnp.mean(d * d, axis=-1, keepdims=True)
    return d / jnp.sqrt(v + _EPS)


def _dot(a, b):
    return jnp.dot(a, b, preferred_element_type=jnp.float32)


def _dot_nt(a, b):
    return jax.lax.dot_general(
        a, b, (((1,), (1,)), ((), ())), preferred_element_type=jnp.float32
    )


def _wait_all(buf, sem):
    pltpu.make_async_copy(buf, buf, sem).wait()


def _loop(lo, hi, fn):
    jax.lax.fori_loop(lo, hi, lambda i, carry: fn(i), None)


def _tile(i, n):
    return pl.ds(i * n if isinstance(i, int) else pl.multiple_of(i * n, n), n)


def _body(
    x_hbm, kt_hbm, vt_hbm, wq_hbm, wo_hbm, wr_hbm, wg_hbm, wu_hbm, wd_hbm,
    out_ref,
    kbuf, vbuf, wqbuf, wobuf, wgbuf, wubuf, wdbuf, xbuf, wrbuf,
    q_scr, qd_scr, s_scr, first_scr, p_scr, l_scr, acc_scr, o_scr, h_scr,
    ksem, vsem, dsem, wqsem, wosem, wgsem, wusem, xsem, wrsem,
    *, B, H, Dh, Sk, D, F,
):
    P = _HG * Dh
    BR = _NB * _RB
    n_hg = H // _HG
    n_groups = B * n_hg
    n_blocks = 3 * n_groups
    n_bands = n_blocks * _NB
    per_row = _NS * 8 // _RB
    scale = Dh ** -0.5
    bf16 = jnp.bfloat16

    def slots(j):
        return j % 2, jnp.where(j == 0, 2, j % 2)

    def issue_block(j, t, k_split=_NB, v_split=0):
        i = t // per_row
        k_slot, v_slot = slots(j)
        streams = (
            (kt_hbm, kbuf, ksem, k_slot, 8 * i + _K_SHIFT, k_split, (0, -n_bands)),
            (vt_hbm, vbuf, vsem, v_slot, 8 * i + _RB - _V_SHIFT, v_split, (n_bands - 1, -1)),
        )
        n_cols = Sk // _CW // per_row
        for c in range(n_cols):
            cols = _tile(t % per_row * n_cols + c, _CW)
            for n in range(0, _NB, 2):
                for queue, (src, dst, sem, slot, r, split, wrap) in enumerate(streams):
                    mid = min(max(split, n), n + 2)
                    for lo, hi, shift in ((n, mid, wrap[0]), (mid, n + 2, wrap[1])):
                        if lo < hi:
                            bands = pl.ds(j * _NB + r // _RB + shift + lo, hi - lo)
                            pltpu.make_async_copy(
                                src.at[bands, _tile(r % _RB // 8, 8), cols],
                                dst.at[slot, pl.ds(lo, hi - lo), _tile(i, 8), cols],
                                sem.at[slot],
                            ).start(priority=queue)

    def issue_edge(j, t):
        rows = [8 * (u // per_row) for u in range(_NS)]
        if j == 0:
            splits = [(_NB, int(r < _V_SHIFT)) for r in rows]
        else:
            splits = [(_NB - (r + _K_SHIFT) // _RB, 0) for r in rows]
        for split in sorted(set(splits)):
            steps = [u for u in range(_NS) if splits[u] == split]
            pl.when((t >= steps[0]) & (t <= steps[-1]))(
                functools.partial(issue_block, j, t, *split)
            )

    def issue_halves(src, dst, sem, cw, i):
        n = src.shape[0] // 2
        for c in range(0, src.shape[2], cw):
            for queue in range(2):
                idx = (pl.ds(queue * n, n), _tile(i, 8), pl.ds(c, cw))
                pltpu.make_async_copy(src.at[idx], dst.at[idx], sem).start(priority=queue)

    def issue_gate_up(i):
        for c in range(0, F, _GU_CW):
            idx = (slice(None), _tile(i, 8), pl.ds(c, _GU_CW))
            pltpu.make_async_copy(wg_hbm.at[idx], wgbuf.at[idx], wgsem).start(priority=0)
            pltpu.make_async_copy(wu_hbm.at[idx], wubuf.at[idx], wusem).start(priority=1)

    def issue_weights(t):
        n_wo, n_gu, rest = wobuf.shape[1] // 8, wgbuf.shape[1] // 8, _NS - _WO_STEPS
        _loop(
            jnp.minimum(t, _WO_STEPS) * n_wo // _WO_STEPS,
            jnp.minimum(t + 1, _WO_STEPS) * n_wo // _WO_STEPS,
            functools.partial(issue_halves, wo_hbm, wobuf, wosem, D),
        )
        _loop(
            jnp.maximum(t - _WO_STEPS, 0) * n_gu // rest,
            jnp.maximum(t + 1 - _WO_STEPS, 0) * n_gu // rest,
            issue_gate_up,
        )

    def issue_down(f):
        half = wdbuf.shape[1] // 2
        for r in range(0, half, _WD_ROWS):
            for queue in range(2):
                idx = (f, pl.ds(queue * half + r, _WD_ROWS))
                pltpu.make_async_copy(wd_hbm.at[idx], wdbuf.at[idx], dsem.at[f]).start(
                    priority=queue
                )

    x_cp = pltpu.make_async_copy(x_hbm, xbuf, xsem)
    wr_cp = pltpu.make_async_copy(wr_hbm, wrbuf, wrsem)
    issue_wq = functools.partial(issue_halves, wq_hbm, wqbuf, wqsem, _WQ_CW)
    _loop(0, 2, issue_wq)
    x_cp.start()
    wr_cp.start(priority=1)
    _loop(2, wqbuf.shape[1] // 8, issue_wq)

    x_cp.wait()
    x = xbuf[...].astype(jnp.float32)
    x = jnp.concatenate([x, x], axis=0)
    xn = _layernorm(x).astype(bf16)
    row = jax.lax.broadcasted_iota(jnp.int32, (_HG, BR), 0)
    col = jax.lax.broadcasted_iota(jnp.int32, (_HG, BR), 1)

    def owners(first):
        d = col + first - row * Dh
        return ((d >= 0) & (d < Dh)) | (d >= P) | (d < Dh - P)

    def roll_rows(a, shift):
        cols = jax.lax.broadcasted_iota(jnp.int32, a.shape, 1)
        a = pltpu.roll(a, P - shift, 1)
        return jnp.where(cols < P - shift, a, pltpu.roll(a, n_groups - 1, 0))

    def project(i):
        _loop(i * _NS // n_hg, (i + 1) * _NS // n_hg, functools.partial(issue_edge, 0))
        pl.when(i == 0)(lambda: _wait_all(wqbuf, wqsem))
        q = _dot(xn, wqbuf[:, :, _tile(i, P)].reshape(D, P))
        for b in range(B):
            o_scr[pl.ds(b * n_hg + i, 1), :] = q[b:b + 1]

    _loop(0, n_hg, project)
    q = roll_rows(o_scr[...], _K_SHIFT)
    for m in range(3):
        q_scr[m] = q[:, m * BR:(m + 1) * BR]
    s_scr[...] = jnp.zeros_like(s_scr)

    def softmax(s):
        s = s * scale
        e = jnp.exp(s - jnp.max(s, axis=-1, keepdims=True))
        p_scr[...] = e
        l_scr[...] = jnp.sum(e, axis=-1, keepdims=True)

    def block(j):
        k_slot, v_slot = slots(j)
        m = j % 3

        def issue(t):
            pl.when(j < n_blocks - 2)(lambda: issue_block(j + 1, t))
            pl.when(j == n_blocks - 2)(lambda: issue_edge(n_blocks - 1, t))
            pl.when(j == n_blocks - 1)(lambda: issue_weights(t))

        _loop(0, 3, issue)
        first = _K_SHIFT + m * BR
        qd_scr[...] = jnp.where(owners(first), q_scr[m, pl.ds(j // 3, 1), :], 0.0)
        start = row[:, :1] * Dh - first
        new_head = ((start >= 0) & (start < BR)) | (start + P < BR)
        _wait_all(kbuf.at[k_slot], ksem.at[k_slot])

        def scores(i):
            cols = _tile(i, Sk // 4)
            s = _dot(qd_scr[...].astype(bf16), kbuf[k_slot, :, :, cols].reshape(BR, Sk // 4))
            s_scr[:, cols] = jnp.where(new_head, 0.0, s_scr[:, cols]) + s
            issue(3 + i)

        _loop(0, 4, scores)
        softmax(s_scr[...])

        @pl.when(j == 0)
        def _():
            first_scr[...] = s_scr[...]

        acc_scr[...] = jnp.zeros_like(acc_scr)
        _wait_all(vbuf.at[v_slot], vsem.at[v_slot])

        def values(i):
            issue(7 + i)
            cols = _tile(i, Sk // 8)
            v = vbuf[v_slot, :, :, cols].reshape(BR, Sk // 8)
            acc_scr[...] += _dot_nt(p_scr[:, cols].astype(bf16), v)

        _loop(0, 8, values)
        _loop(15, _NS, issue)
        o = jnp.where(owners(m * BR - _V_SHIFT), acc_scr[...] / l_scr[...], 0.0)
        o = jnp.sum(o, axis=0, keepdims=True)
        for u in range(3):

            @pl.when(m == u)
            def _(u=u):
                o_scr[pl.ds(j // 3, 1), u * BR:(u + 1) * BR] = o

    _loop(0, n_blocks, block)

    s, s_first = s_scr[...], first_scr[...]
    softmax(jnp.where(row[:, :1] == 0, s + s_first, jnp.where(row[:, :1] == _HG - 1, s, s_first)))
    n = Dh + _RB
    v = vbuf[2, :n // _RB].reshape(n, Sk)
    issue_down(0)
    o = _dot_nt(p_scr[...].astype(bf16), v) / l_scr[...]
    o_scr[:1, :n] = jnp.sum(jnp.where(owners(-_V_SHIFT)[:, :n], o, 0.0), axis=0, keepdims=True)
    o_scr[...] = roll_rows(o_scr[...], _V_SHIFT)

    _wait_all(wobuf, wosem)
    h_scr[...] = x
    n = _WO_BANDS // n_hg
    for i in range(n_hg):
        o = jnp.concatenate([o_scr[pl.ds(b % B * n_hg + i, 1), :] for b in range(2 * B)], axis=0)
        h_scr[...] += _dot(o.astype(bf16), wobuf[i * n:(i + 1) * n].reshape(P, D))
        if i + 1 < n_hg:
            issue_down(i + 1)

    h = h_scr[...]
    hn = _layernorm(h)
    hb = hn.astype(bf16)
    wr_cp.wait()
    r = jnp.sum(hn * wrbuf[...].astype(jnp.float32).reshape(1, D), axis=-1, keepdims=True)
    route = jax.nn.sigmoid(r)
    _wait_all(wgbuf, wgsem)
    _wait_all(wubuf, wusem)
    gate = _dot(hb, wgbuf[...].reshape(D, F))
    up = _dot(hb, wubuf[...].reshape(D, F))
    act = (gate * jax.nn.sigmoid(gate) * up).astype(bf16)
    y = jnp.zeros((2 * B, D), jnp.float32)
    n = F // n_hg
    for f in range(n_hg):
        _wait_all(wdbuf.at[f], dsem.at[f])
        y = y + _dot(act[:, f * n:(f + 1) * n], wdbuf[f])
    out = h + (hn + (hn * 0.0 + y * route))
    out_ref[...] = out[:B].astype(out_ref.dtype)


@jax.jit
def pallas_sequential_preLN__mha_block_cached__moe_arch_mod__decode_kernel(
    A_x: jax.Array,
    A_k_cache: jax.Array,
    A_v_cache: jax.Array,
    A_wq: jax.Array,
    A_wo: jax.Array,
    B_x: jax.Array,
    B_w_r: jax.Array,
    B_w_gate: jax.Array,
    B_w_up: jax.Array,
    B_w_down: jax.Array,
):
    del B_x
    B, Sq, D = A_x.shape
    _, H, Sk, Dh = A_k_cache.shape
    F = B_w_gate.shape[1]
    P = _HG * Dh
    n_hg = H // _HG
    assert Sq == 1 and B == 4 and H % _HG == 0 and P == 3 * _NB * _RB and Sk % (2 * _CW) == 0
    assert 0 < _V_SHIFT <= _RB and Dh - _V_SHIFT <= _K_SHIFT <= Dh
    assert F % (2 * n_hg * _WD_ROWS) == 0
    dt = A_k_cache.dtype
    f32 = jnp.float32

    kt = jnp.swapaxes(A_k_cache, 2, 3).reshape(-1, _RB, Sk)
    vt = jnp.swapaxes(A_v_cache, 2, 3).reshape(-1, _RB, Sk)
    wq = A_wq.reshape(_WQ_BANDS, -1, H * Dh)
    wo = A_wo.reshape(_WO_BANDS, -1, D)
    wg = B_w_gate.reshape(_GU_BANDS, -1, F)
    wu = B_w_up.reshape(_GU_BANDS, -1, F)
    wd = B_w_down.reshape(n_hg, -1, D)

    out = pl.pallas_call(
        functools.partial(_body, B=B, H=H, Dh=Dh, Sk=Sk, D=D, F=F),
        in_specs=[pl.BlockSpec(memory_space=pl.ANY)] * 9,
        out_specs=pl.BlockSpec(memory_space=pltpu.VMEM),
        out_shape=jax.ShapeDtypeStruct((B, D), A_x.dtype),
        scratch_shapes=[
            pltpu.VMEM((2, _NB, _RB, Sk), dt),
            pltpu.VMEM((3, _NB, _RB, Sk), dt),
            *[pltpu.VMEM(w.shape, dt) for w in (wq, wo, wg, wu, wd)],
            pltpu.VMEM((B, D), dt),
            pltpu.VMEM((D,), dt),
            pltpu.VMEM((3, B * n_hg, P // 3), f32),
            pltpu.VMEM((_HG, P // 3), f32),
            *[pltpu.VMEM((_HG, Sk), f32)] * 3,
            pltpu.VMEM((_HG, 1), f32),
            pltpu.VMEM((_HG, P // 3), f32),
            pltpu.VMEM((B * n_hg, P), f32),
            pltpu.VMEM((2 * B, D), f32),
            pltpu.SemaphoreType.DMA((2,)),
            pltpu.SemaphoreType.DMA((3,)),
            pltpu.SemaphoreType.DMA((n_hg,)),
            *[pltpu.SemaphoreType.DMA(())] * 6,
        ],
        compiler_params=pltpu.CompilerParams(vmem_limit_bytes=100 * 1024 * 1024),
    )(A_x.reshape(B, D), kt, vt, wq, wo, B_w_r, wg, wu, wd)
    return out.reshape(B, Sq, D)
```

```python
import functools

import jax
import jax.numpy as jnp
import jax.experimental.pallas as pl
import jax.experimental.pallas.tpu as pltpu

_EPS = 1e-5
_HG = 8
_RB = 64
_NB = 8
_CW = 1024
_K_SHIFT = 176
_V_SHIFT = 40
_WQ_BANDS, _WQ_CW = 10, 384
_WO_BANDS = 8
_GU_BANDS, _GU_CW = 4, 512
_WD_ROWS = 24
_NS = 16
_WO_STEPS = 11


def _layernorm(x):
    m = jnp.mean(x, axis=-1, keepdims=True)
    d = x - m
    v = jnp.mean(d * d, axis=-1, keepdims=True)
    return d / jnp.sqrt(v + _EPS)


def _dot(a, b):
    return jnp.dot(a, b, preferred_element_type=jnp.float32)


def _dot_nt(a, b):
    return jax.lax.dot_general(
        a, b, (((1,), (1,)), ((), ())), preferred_element_type=jnp.float32
    )


def _wait_all(buf, sem):
    pltpu.make_async_copy(buf, buf, sem).wait()


def _loop(lo, hi, fn):
    jax.lax.fori_loop(lo, hi, lambda i, carry: fn(i), None)


def _tile(i, n):
    return pl.ds(i * n if isinstance(i, int) else pl.multiple_of(i * n, n), n)


def _body(
    x_hbm, kt_hbm, vt_hbm, wq_hbm, wo_hbm, wr_hbm, wg_hbm, wu_hbm, wd_hbm,
    out_ref,
    kbuf, vbuf, wqbuf, wobuf, wgbuf, wubuf, wdbuf, xbuf, wrbuf,
    q_scr, qd_scr, s_scr, first_scr, p_scr, l_scr, acc_scr, o_scr, h_scr,
    ksem, vsem, dsem, wqsem, wosem, wgsem, wusem, xsem, wrsem,
    *, B, H, Dh, Sk, D, F,
):
    P = _HG * Dh
    BR = _NB * _RB
    n_hg = H // _HG
    n_groups = B * n_hg
    n_blocks = 3 * n_groups
    per_row = _NS * 8 // _RB
    scale = Dh ** -0.5
    bf16 = jnp.bfloat16

    def slots(j):
        return j % 2, jnp.where(j == 0, 2, j % 2)

    def issue_block(j, t, k_split=_NB, v_split=0):
        i = t // per_row
        k_slot, v_slot = slots(j)
        n_cols = Sk // _CW // per_row

        def issue(src, dst, sem, queue, cols, n, r, shift, split, wraps):
            n_bands, rb = src.shape[:2]
            band = j * (BR // rb) + (r + shift + rb) // rb - 1
            mid = min(max(split, n), n + 2)
            for lo, hi, wrap in ((n, mid, wraps[0]), (mid, n + 2, wraps[1])):
                if lo < hi:
                    bands = pl.ds(band + lo + wrap * n_bands, hi - lo)
                    pltpu.make_async_copy(
                        src.at[bands, _tile((r + shift + rb) % rb // 8, 8), cols],
                        dst.at[pl.ds(lo, hi - lo), _tile(r // 8, 8), cols],
                        sem,
                    ).start(priority=queue)

        for c in range(n_cols):
            cols = _tile(t % per_row * n_cols + c, _CW)
            for u in range(_NB // 2):
                issue(
                    kt_hbm, kbuf.at[k_slot], ksem.at[k_slot], 0, cols,
                    2 * u, 8 * i, _K_SHIFT, k_split, (0, -1),
                )
                issue(
                    vt_hbm, vbuf.at[v_slot], vsem.at[v_slot], 1, cols,
                    u // 2 * 2, 8 * i + u % 2 * _RB, -_V_SHIFT, 0 if u % 2 else v_split, (1, 0),
                )

    def issue_edge(j, t):
        rows = [8 * (u // per_row) for u in range(_NS)]
        if j == 0:
            splits = [(_NB, int(r < _V_SHIFT)) for r in rows]
        else:
            splits = [(_NB - (r + _K_SHIFT) // _RB, 0) for r in rows]
        for split in sorted(set(splits)):
            steps = [u for u in range(_NS) if splits[u] == split]
            pl.when((t >= steps[0]) & (t <= steps[-1]))(
                functools.partial(issue_block, j, t, *split)
            )

    def issue_halves(src, dst, sem, cw, i):
        n = src.shape[0] // 2
        for c in range(0, src.shape[2], cw):
            for queue in range(2):
                idx = (pl.ds(queue * n, n), _tile(i, 8), pl.ds(c, cw))
                pltpu.make_async_copy(src.at[idx], dst.at[idx], sem).start(priority=queue)

    def issue_gate_up(i):
        for c in range(0, F, _GU_CW):
            idx = (slice(None), _tile(i, 8), pl.ds(c, _GU_CW))
            pltpu.make_async_copy(wg_hbm.at[idx], wgbuf.at[idx], wgsem).start(priority=0)
            pltpu.make_async_copy(wu_hbm.at[idx], wubuf.at[idx], wusem).start(priority=1)

    def issue_weights(t):
        n_wo, n_gu, rest = wobuf.shape[1] // 8, wgbuf.shape[1] // 8, _NS - _WO_STEPS
        _loop(
            jnp.minimum(t, _WO_STEPS) * n_wo // _WO_STEPS,
            jnp.minimum(t + 1, _WO_STEPS) * n_wo // _WO_STEPS,
            functools.partial(issue_halves, wo_hbm, wobuf, wosem, D),
        )
        _loop(
            jnp.maximum(t - _WO_STEPS, 0) * n_gu // rest,
            jnp.maximum(t + 1 - _WO_STEPS, 0) * n_gu // rest,
            issue_gate_up,
        )

    def issue_down(f):
        half = wdbuf.shape[1] // 2
        for r in range(0, half, _WD_ROWS):
            for queue in range(2):
                idx = (f, pl.ds(queue * half + r, _WD_ROWS))
                pltpu.make_async_copy(wd_hbm.at[idx], wdbuf.at[idx], dsem.at[f]).start(
                    priority=queue
                )

    x_cp = pltpu.make_async_copy(x_hbm, xbuf, xsem)
    wr_cp = pltpu.make_async_copy(wr_hbm, wrbuf, wrsem)
    issue_wq = functools.partial(issue_halves, wq_hbm, wqbuf, wqsem, _WQ_CW)
    _loop(0, 2, issue_wq)
    x_cp.start()
    wr_cp.start(priority=1)
    _loop(2, wqbuf.shape[1] // 8, issue_wq)

    x_cp.wait()
    x = xbuf[...].astype(jnp.float32)
    x = jnp.concatenate([x, x], axis=0)
    xn = _layernorm(x).astype(bf16)
    row = jax.lax.broadcasted_iota(jnp.int32, (_HG, BR), 0)
    col = jax.lax.broadcasted_iota(jnp.int32, (_HG, BR), 1)

    def owners(first):
        d = col + first - row * Dh
        return ((d >= 0) & (d < Dh)) | (d >= P) | (d < Dh - P)

    def roll_rows(a, shift):
        cols = jax.lax.broadcasted_iota(jnp.int32, a.shape, 1)
        a = pltpu.roll(a, P - shift, 1)
        return jnp.where(cols < P - shift, a, pltpu.roll(a, n_groups - 1, 0))

    def project(i):
        _loop(i * _NS // n_hg, (i + 1) * _NS // n_hg, functools.partial(issue_edge, 0))
        pl.when(i == 0)(lambda: _wait_all(wqbuf, wqsem))
        q = _dot(xn, wqbuf[:, :, _tile(i, P)].reshape(D, P))
        for b in range(B):
            o_scr[pl.ds(b * n_hg + i, 1), :] = q[b:b + 1]

    _loop(0, n_hg, project)
    q = roll_rows(o_scr[...], _K_SHIFT)
    for m in range(3):
        q_scr[m] = q[:, m * BR:(m + 1) * BR]
    s_scr[...] = jnp.zeros_like(s_scr)

    def softmax(s):
        s = s * scale
        e = jnp.exp(s - jnp.max(s, axis=-1, keepdims=True))
        p_scr[...] = e
        l_scr[...] = jnp.sum(e, axis=-1, keepdims=True)

    def block(j):
        k_slot, v_slot = slots(j)
        m = j % 3

        def issue(t):
            pl.when(j < n_blocks - 2)(lambda: issue_block(j + 1, t))
            pl.when(j == n_blocks - 2)(lambda: issue_edge(n_blocks - 1, t))
            pl.when(j == n_blocks - 1)(lambda: issue_weights(t))

        _loop(0, 3, issue)
        first = _K_SHIFT + m * BR
        qd_scr[...] = jnp.where(owners(first), q_scr[m, pl.ds(j // 3, 1), :], 0.0)
        start = row[:, :1] * Dh - first
        new_head = ((start >= 0) & (start < BR)) | (start + P < BR)
        _wait_all(kbuf.at[k_slot], ksem.at[k_slot])

        def scores(i):
            cols = _tile(i, Sk // 4)
            s = _dot(qd_scr[...].astype(bf16), kbuf[k_slot, :, :, cols].reshape(BR, Sk // 4))
            s_scr[:, cols] = jnp.where(new_head, 0.0, s_scr[:, cols]) + s
            issue(3 + i)

        _loop(0, 4, scores)
        softmax(s_scr[...])

        @pl.when(j == 0)
        def _():
            first_scr[...] = s_scr[...]

        acc_scr[...] = jnp.zeros_like(acc_scr)
        _wait_all(vbuf.at[v_slot], vsem.at[v_slot])

        def values(i):
            issue(7 + i)
            cols = _tile(i, Sk // 8)
            v = vbuf[v_slot, :, :, cols].reshape(BR, Sk // 8)
            acc_scr[...] += _dot_nt(p_scr[:, cols].astype(bf16), v)

        _loop(0, 8, values)
        _loop(15, _NS, issue)
        o = jnp.where(owners(m * BR - _V_SHIFT), acc_scr[...] / l_scr[...], 0.0)
        o = jnp.sum(o, axis=0, keepdims=True)
        for u in range(3):

            @pl.when(m == u)
            def _(u=u):
                o_scr[pl.ds(j // 3, 1), u * BR:(u + 1) * BR] = o

    _loop(0, n_blocks, block)

    s, s_first = s_scr[...], first_scr[...]
    softmax(jnp.where(row[:, :1] == 0, s + s_first, jnp.where(row[:, :1] == _HG - 1, s, s_first)))
    n = Dh + _RB
    v = vbuf[2, :n // (2 * _RB)].reshape(n, Sk)
    issue_down(0)
    o = _dot_nt(p_scr[...].astype(bf16), v) / l_scr[...]
    o_scr[:1, :n] = jnp.sum(jnp.where(owners(-_V_SHIFT)[:, :n], o, 0.0), axis=0, keepdims=True)
    o_scr[...] = roll_rows(o_scr[...], _V_SHIFT)

    _wait_all(wobuf, wosem)
    h_scr[...] = x
    n = _WO_BANDS // n_hg
    for i in range(n_hg):
        o = jnp.concatenate([o_scr[pl.ds(b % B * n_hg + i, 1), :] for b in range(2 * B)], axis=0)
        h_scr[...] += _dot(o.astype(bf16), wobuf[i * n:(i + 1) * n].reshape(P, D))
        if i + 1 < n_hg:
            issue_down(i + 1)

    h = h_scr[...]
    hn = _layernorm(h)
    hb = hn.astype(bf16)
    wr_cp.wait()
    r = jnp.sum(hn * wrbuf[...].astype(jnp.float32).reshape(1, D), axis=-1, keepdims=True)
    route = jax.nn.sigmoid(r)
    _wait_all(wgbuf, wgsem)
    _wait_all(wubuf, wusem)
    gate = _dot(hb, wgbuf[...].reshape(D, F))
    up = _dot(hb, wubuf[...].reshape(D, F))
    act = (gate * jax.nn.sigmoid(gate) * up).astype(bf16)
    y = jnp.zeros((2 * B, D), jnp.float32)
    n = F // n_hg
    for f in range(n_hg):
        _wait_all(wdbuf.at[f], dsem.at[f])
        y = y + _dot(act[:, f * n:(f + 1) * n], wdbuf[f])
    out = h + (hn + (hn * 0.0 + y * route))
    out_ref[...] = out[:B].astype(out_ref.dtype)


@jax.jit
def pallas_sequential_preLN__mha_block_cached__moe_arch_mod__decode_kernel(
    A_x: jax.Array,
    A_k_cache: jax.Array,
    A_v_cache: jax.Array,
    A_wq: jax.Array,
    A_wo: jax.Array,
    B_x: jax.Array,
    B_w_r: jax.Array,
    B_w_gate: jax.Array,
    B_w_up: jax.Array,
    B_w_down: jax.Array,
):
    del B_x
    B, Sq, D = A_x.shape
    _, H, Sk, Dh = A_k_cache.shape
    F = B_w_gate.shape[1]
    P = _HG * Dh
    n_hg = H // _HG
    assert Sq == 1 and B == 4 and H % _HG == 0 and P == 3 * _NB * _RB and Sk % (2 * _CW) == 0
    assert 0 < _V_SHIFT <= _RB and Dh - _V_SHIFT <= _K_SHIFT <= Dh
    assert F % (2 * n_hg * _WD_ROWS) == 0
    dt = A_k_cache.dtype
    f32 = jnp.float32

    kt = jnp.swapaxes(A_k_cache, 2, 3).reshape(-1, _RB, Sk)
    vt = jnp.swapaxes(A_v_cache, 2, 3).reshape(-1, 2 * _RB, Sk)
    wq = A_wq.reshape(_WQ_BANDS, -1, H * Dh)
    wo = A_wo.reshape(_WO_BANDS, -1, D)
    wg = B_w_gate.reshape(_GU_BANDS, -1, F)
    wu = B_w_up.reshape(_GU_BANDS, -1, F)
    wd = B_w_down.reshape(n_hg, -1, D)

    out = pl.pallas_call(
        functools.partial(_body, B=B, H=H, Dh=Dh, Sk=Sk, D=D, F=F),
        in_specs=[pl.BlockSpec(memory_space=pl.ANY)] * 9,
        out_specs=pl.BlockSpec(memory_space=pltpu.VMEM),
        out_shape=jax.ShapeDtypeStruct((B, D), A_x.dtype),
        scratch_shapes=[
            pltpu.VMEM((2, _NB, _RB, Sk), dt),
            pltpu.VMEM((3, _NB // 2, 2 * _RB, Sk), dt),
            *[pltpu.VMEM(w.shape, dt) for w in (wq, wo, wg, wu, wd)],
            pltpu.VMEM((B, D), dt),
            pltpu.VMEM((D,), dt),
            pltpu.VMEM((3, B * n_hg, P // 3), f32),
            pltpu.VMEM((_HG, P // 3), f32),
            *[pltpu.VMEM((_HG, Sk), f32)] * 3,
            pltpu.VMEM((_HG, 1), f32),
            pltpu.VMEM((_HG, P // 3), f32),
            pltpu.VMEM((B * n_hg, P), f32),
            pltpu.VMEM((2 * B, D), f32),
            pltpu.SemaphoreType.DMA((2,)),
            pltpu.SemaphoreType.DMA((3,)),
            pltpu.SemaphoreType.DMA((n_hg,)),
            *[pltpu.SemaphoreType.DMA(())] * 6,
        ],
        compiler_params=pltpu.CompilerParams(vmem_limit_bytes=100 * 1024 * 1024),
    )(A_x.reshape(B, D), kt, vt, wq, wo, B_w_r, wg, wu, wd)
    return out.reshape(B, Sq, D)
```
